```python
import os as _os
_os.environ.setdefault("JAX_PLATFORMS", "cpu")
import jax
import jax.numpy as jnp

def _softmax(x, axis=-1):
    return jax.nn.softmax(x, axis=axis)
def _gelu(x):
    return jax.nn.gelu(x, approximate=True)
def _silu(x):
    return jax.nn.silu(x)
def _sigmoid(x):
    return jax.nn.sigmoid(x)
def _layernorm(x, axis=-1, eps=1e-5):
    m = jnp.mean(x, axis=axis, keepdims=True)
    v = jnp.var(x, axis=axis, keepdims=True)
    return (x - m) / jnp.sqrt(v + eps)
def _scatter_add(tgt, idx, src, axis=0):
    return tgt.at[idx].add(src)
def _segment_sum(src, seg, n):
    return jax.ops.segment_sum(src, seg, n)
class _Rng:
    def __init__(self, key):
        self._k = key
    def _next(self):
        self._k, sub = jax.random.split(self._k)
        return sub
    def normal(self, shape):
        return jax.random.normal(self._next(), shape, dtype=jnp.bfloat16)
    def randint(self, lo, hi, shape):
        return jax.random.randint(self._next(), shape, lo, hi, dtype=jnp.int32)
    def uniform(self, shape, lo=0.0, hi=1.0):
        return jax.random.uniform(self._next(), shape, jnp.bfloat16, lo, hi)
    def permutation(self, n):
        return jax.random.permutation(self._next(), n)


kernel_name = 'concat_heads__compressed_kv_cla__gqa_block_cached__decode'

def setup_inputs():
    _rng = _Rng(jax.random.key(int.from_bytes(__import__("os").urandom(4), "little")))
    _w = (lambda a: (lambda t: t.astype(jnp.bfloat16) if jnp.issubdtype(t.dtype, jnp.floating) else t)(jnp.asarray(a)))
    def _A_setup():
        B, H, Sq, Sk, D, M = 4, 32, 1, 4096, 128, 512
        Dc = 4 * D
        return {
            "x": _w((lambda *s: _rng.normal(s) * 3.2)(B, Sq, M)),
            "c_kv": _w((lambda *s: _rng.normal(s) * 0.05)(B, Sk, Dc)),
            "w_q": _w((lambda *s: _rng.normal(s) * 3.2)(M, H, D) * (M ** -0.5)),
            "w_uk": _w((lambda *s: _rng.normal(s) * 3.2)(Dc, H, D) * (Dc ** -0.5)),
            "w_uv": _w((lambda *s: _rng.normal(s) * 0.05)(Dc, H, D) * (Dc ** -0.5)),
            "w_o": _w((lambda *s: _rng.normal(s) * 0.05)(H, D, M) * ((H * D) ** -0.5)),
        }
    _A_in = _A_setup()

    def _B_setup():
        B, Sq, D = 4, 1, 512
        Hq, Hkv, Sk, Dh = 32, 8, 4096, 128
        assert Hq % Hkv == 0, (Hq, Hkv)
        return {
            "x": _w((lambda *s: _rng.normal(s) * 0.8)(B, Sq, D)),
            "k_cache": _w((lambda *s: _rng.normal(s) * 0.8)(B, Hkv, Sk, Dh)),
            "v_cache": _w((lambda *s: _rng.normal(s) * 0.05)(B, Hkv, Sk, Dh)),
            "wq": _w((lambda *s: _rng.normal(s) * 0.8)(D, Hq * Dh) * (D ** -0.5)),
            "wo": _w((lambda *s: _rng.normal(s) * 0.05)(Hq * Dh, D) * ((Hq * Dh) ** -0.5)),
        }
    _B_in = _B_setup()

    return {
        "A_x": _A_in["x"],
        "A_c_kv": _A_in["c_kv"],
        "A_w_q": _A_in["w_q"],
        "A_w_uk": _A_in["w_uk"],
        "A_w_uv": _A_in["w_uv"],
        "A_w_o": _A_in["w_o"],
        "B_x": _B_in["x"],
        "B_k_cache": _B_in["k_cache"],
        "B_v_cache": _B_in["v_cache"],
        "B_wq": _B_in["wq"],
        "B_wo": _B_in["wo"],
    }

def reference(A_x, A_c_kv, A_w_q, A_w_uk, A_w_uv, A_w_o, B_x, B_k_cache, B_v_cache, B_wq, B_wo):
    def _A_ref(x, c_kv, w_q, w_uk, w_uv, w_o):
        B, Sq, M = x.shape[0], x.shape[1], x.shape[2]
        Sk = c_kv.shape[1]
        H, D = w_q.shape[1], w_q.shape[2]
        q = jnp.einsum("bqm,mhd->bhqd", x, w_q)
        k = jnp.einsum("bkc,chd->bhkd", c_kv, w_uk)
        v = jnp.einsum("bkc,chd->bhkd", c_kv, w_uv)
        scores = jnp.einsum("bhqd,bhkd->bhqk", q, k) * (D ** -0.5)
        off = Sk - Sq
        qi = jnp.arange(Sq)[:, None]
        kj = jnp.arange(Sk)[None, :]
        cmask = kj <= (qi + off)
        scores = jnp.where(cmask[None, None], scores, -1e9)
        p = _softmax(scores, axis=-1)
        ctx = jnp.einsum("bhqk,bhkd->bhqd", p, v)
        return jnp.einsum("bhqd,hdm->bqm", ctx, w_o)

    def _B_ref(x, k_cache, v_cache, wq, wo):
        B, Sq, D = x.shape
        Hq, Dh = 32, 128
        Hkv = k_cache.shape[1]
        rep = Hq // Hkv
        q = (lambda x, *d: x.transpose(*d))((x @ wq).reshape(B, Sq, Hq, Dh), 0, 2, 1, 3)
        k = jnp.repeat(k_cache, rep, axis=1)
        v = jnp.repeat(v_cache, rep, axis=1)
        scores = jnp.einsum("bhqd,bhkd->bhqk", q, k) * (Dh ** -0.5)
        p = _softmax(scores, axis=-1)
        o = jnp.einsum("bhqk,bhkd->bhqd", p, v)
        return (lambda x, *d: x.transpose(*d))(o, 0, 2, 1, 3).reshape(B, Sq, Hq * Dh) @ wo

    a = _A_ref(A_x, A_c_kv, A_w_q, A_w_uk, A_w_uv, A_w_o)
    b = _B_ref(B_x, B_k_cache, B_v_cache, B_wq, B_wo)
    return jnp.concatenate([a, b], axis=-1)
```

```python
import jax
import jax.numpy as jnp
from jax import lax
import jax.experimental.pallas as pl
import jax.experimental.pallas.tpu as pltpu

_NT = (((1,), (1,)), ((), ()))
_F32 = jnp.float32
_BF16 = jnp.bfloat16
_LOOK = 4
_MAXG = 3


def _dot(a, b):
    return jnp.dot(a, b, preferred_element_type=_F32)


def _dot_nt(a, b):
    return lax.dot_general(a, b, _NT, preferred_element_type=_F32)


def _kernel(xa_hbm, c_hbm, wq_hbm, wuk_hbm, wuv_hbm, woa_hbm,
            xb_hbm, k_hbm, v_hbm, wqb_hbm, wob_hbm,
            out_ref,
            xa_buf, xb_buf, wq_buf, wuk_buf, wuv_buf, woa_buf, wqb_buf, wob_buf,
            c_buf, k_buf, v_buf,
            qa_s, qabs_s, qabs_t, qb_s, qb_t, sa_s, sb_s, ob_s, cc_s, ctx_s,
            hsem, lsem, xsem):
    scale = 128 ** -0.5

    def sems(t, g):
        i = (t % _LOOK) * _MAXG + g
        return hsem.at[i], lsem.at[i]

    def pair(src, dst, t, g):
        hs, ls = sems(t, g)
        hi = pltpu.make_async_copy(src(0, 1), dst(0, 1), hs)
        lo = pltpu.make_async_copy(src(1, 3), dst(1, 3), ls)
        return hi, lo

    class Stream:
        def __init__(self, steps, groups, fn):
            self.steps, self.groups, self.fn = steps, groups, fn

        def start(self, t, g):
            hi, lo = self.fn(t, g)
            hi.start(priority=0)
            lo.start(priority=1)

        def wait(self, t, g):
            hi, lo = self.fn(t, g)
            lo.wait()
            hi.wait()

    def rows_fn(hbm, buf, rows):
        def fn(t, g):
            r = pl.ds(pl.multiple_of(t * rows, rows), rows)
            return pair(lambda o, n: hbm.at[pl.ds(4 * g + o, n), r],
                        lambda o, n: buf.at[pl.ds(4 * g + o, n), r], t, g)
        return fn

    def wqb_fn(t, g):
        r = pl.ds(pl.multiple_of((t // 2) * 8, 8), 8)
        c = pl.ds(pl.multiple_of((t % 2) * 2048, 2048), 2048)
        return pair(lambda o, n: wqb_hbm.at[pl.ds(4 * g + o, n), r, c],
                    lambda o, n: wqb_buf.at[pl.ds(4 * g + o, n), r, c], t, g)

    def k_stream(b):
        kfn = rows_fn(k_hbm.at[b], k_buf, 128)

        def fn(t, g):
            if g < 2:
                return kfn(t, g)
            r = pl.ds(pl.multiple_of(t * 32, 32), 32)
            return pair(lambda o, n: c_hbm.at[b, pl.ds(o, n), r],
                        lambda o, n: c_buf.at[t, pl.ds(o, n)], t, g)
        return Stream(32, 3, fn)

    def v_stream(b):
        return Stream(32, 2, rows_fn(v_hbm.at[b], v_buf, 128))

    s_wq = Stream(16, 2, rows_fn(wq_hbm, wq_buf, 128))
    s_wuk = Stream(16, 2, rows_fn(wuk_hbm, wuk_buf, 128))
    s_wqb = Stream(16, 2, wqb_fn)
    s_wuv = Stream(16, 2, rows_fn(wuv_hbm, wuv_buf, 128))
    s_wob = Stream(16, 2, rows_fn(wob_hbm, wob_buf, 32))
    s_woa = Stream(16, 2, rows_fn(woa_hbm, woa_buf, 32))

    def pace(cur, nxt, t, g):
        cur.wait(t, g)

        @pl.when(t + _LOOK < cur.steps)
        def _():
            cur.start(t + _LOOK, g)

        for cond, st in nxt:
            gs = [g] if g < st.groups else []
            if g == cur.groups - 1:
                gs += list(range(cur.groups, st.groups))
            if not gs:
                continue
            c = t + _LOOK >= cur.steps
            if cond is not None:
                c = jnp.logical_and(c, cond)

            @pl.when(c)
            def _():
                for gg in gs:
                    st.start(t + _LOOK - cur.steps, gg)

    def head_pair(buf, a, s, lo, hi):
        view = buf.bitcast(jnp.uint32).at[:, pl.ds(pl.multiple_of(4 * a, 4), 1012), :]
        x = jnp.concatenate(
            [view[r, pl.ds(s, 64, stride=16), :] for r in range(lo, hi)], axis=0)
        even = pltpu.bitcast(x << 16, _F32).astype(_BF16)
        odd = pltpu.bitcast(x & jnp.uint32(0xFFFF0000), _F32).astype(_BF16)
        return even, odd

    for t in range(_LOOK):
        for g in range(2):
            s_wq.start(t, g)
    cxa = pltpu.make_async_copy(xa_hbm, xa_buf, xsem.at[0])
    cxb = pltpu.make_async_copy(xb_hbm, xb_buf, xsem.at[1])
    cxa.start()
    cxb.start()

    def p0(t, c):
        for g in range(2):
            pace(s_wq, [(None, s_wuk)], t, g)
        return c
    lax.fori_loop(0, 16, p0, 0)
    cxa.wait()
    cxb.wait()
    xa = xa_buf[...]
    xb = xb_buf[...]

    def p1(a, c):
        for s in range(4):
            t = 4 * a + s
            pace(s_wuk, [(None, s_wqb)], t, 0)
            ev, od = head_pair(wq_buf, a, s, 0, 8)
            qa_s[2 * t] = _dot(xa, ev)
            qa_s[2 * t + 1] = _dot(xa, od)
            pace(s_wuk, [(None, s_wqb)], t, 1)
        return c
    lax.fori_loop(0, 4, p1, 0)

    def p2(a, c):
        for s in range(4):
            t = 4 * a + s
            for g in range(2):
                pace(s_wqb, [(None, s_wuv)], t, g)
                ev, od = head_pair(wuk_buf, a, s, 4 * g, 4 * g + 4)
                for h, w in ((2 * t, ev), (2 * t + 1, od)):
                    r = _dot_nt(qa_s[h].astype(_BF16), w) * scale
                    row = pl.ds(pl.multiple_of(h * 8, 8), 4)
                    qabs_s[2 * g, row, :] = r[:, :128]
                    qabs_s[2 * g + 1, row, :] = r[:, 128:]
        return c
    lax.fori_loop(0, 4, p2, 0)
    for b in range(4):
        qabs_t[b] = jnp.concatenate(
            [qabs_s[ct, pl.ds(b, 32, stride=8), :] for ct in range(4)], axis=1).astype(_BF16)

    def p3(t, c):
        for g in range(2):
            pace(s_wuv, [(None, k_stream(0))], t, g)
            h = 2 * t + g
            w = wqb_buf[:, :, pl.ds(pl.multiple_of(h * 128, 128), 128)].reshape(512, 128)
            q = _dot(xb, w).astype(_BF16).astype(_F32) * scale
            qb_s[pl.ds(pl.multiple_of(h * 8, 8), 4), :] = q
        return c
    lax.fori_loop(0, 16, p3, 0)
    for b in range(4):
        qb_t[b] = qb_s[pl.ds(b, 32, stride=8), :]

    top = lax.broadcasted_iota(jnp.int32, (8, 128), 0) < 4

    def batch(b, carry):
        ks, vs = k_stream(b), v_stream(b)
        qb = [qb_t[b, 8 * i:8 * i + 8, :].astype(_BF16) for i in range(4)]
        qabs = qabs_t[b]

        def kstep(t, c):
            mb, ma = list(c[0]), c[1]
            r = pl.ds(pl.multiple_of(t * 128, 128), 128)
            for g in range(2):
                pace(ks, [(None, vs)], t, g)
                for i in (2 * g, 2 * g + 1):
                    s = jnp.where(top, _dot_nt(qb[i], k_buf[2 * i, r, :]),
                                  _dot_nt(qb[i], k_buf[2 * i + 1, r, :]))
                    sb_s[t, i] = s
                    mb[i] = jnp.maximum(mb[i], s)
            pace(ks, [(None, vs)], t, 2)
            sa = _dot_nt(qabs, c_buf[t].reshape(128, 512))
            sa_s[t] = sa
            return tuple(mb), jnp.maximum(ma, sa)

        ninf = lambda n: jnp.full((n, 128), -jnp.inf, _F32)
        mb, ma = lax.fori_loop(0, 32, kstep, ((ninf(8),) * 4, ninf(32)))
        mb = [jnp.broadcast_to(jnp.max(m, axis=-1, keepdims=True), (8, 128)) for m in mb]
        ma = jnp.broadcast_to(jnp.max(ma, axis=-1, keepdims=True), (32, 128))

        nxt = [(b < 3, k_stream(jnp.minimum(b + 1, 3))), (b == 3, s_wob)]

        def vstep(t, c):
            lb, ab, la, aa = list(c[0]), list(c[1]), c[2], c[3]
            r = pl.ds(pl.multiple_of(t * 128, 128), 128)
            pace(vs, nxt, t, 0)
            pace(vs, nxt, t, 1)
            for i in range(4):
                p = jnp.exp(sb_s[t, i] - mb[i])
                lb[i] = lb[i] + p
                p = p.astype(_BF16)
                ab[i] = ab[i] + jnp.where(top, _dot(p, v_buf[2 * i, r, :]),
                                          _dot(p, v_buf[2 * i + 1, r, :]))
            p = jnp.exp(sa_s[t] - ma)
            la = la + p
            aa = aa + _dot(p.astype(_BF16), c_buf[t].reshape(128, 512))
            return tuple(lb), tuple(ab), la, aa

        z8 = jnp.zeros((8, 128), _F32)
        lb, ab, la, aa = lax.fori_loop(
            0, 32, vstep,
            ((z8,) * 4, (z8,) * 4, jnp.zeros((32, 128), _F32), jnp.zeros((32, 512), _F32)))
        ob = jnp.concatenate(
            [ab[i] / jnp.sum(lb[i], axis=-1, keepdims=True) for i in range(4)], axis=0)
        cc = aa / jnp.sum(la, axis=-1, keepdims=True)
        for bb in range(4):
            @pl.when(b == bb)
            def _():
                ob_s[pl.ds(bb, 32, stride=8), :] = ob
                for ct in range(4):
                    cc_s[ct, pl.ds(bb, 32, stride=8), :] = cc[:, ct * 128:(ct + 1) * 128]
        return carry
    lax.fori_loop(0, 4, batch, 0)

    def proj(lhs_ref, w_buf, j, regions):
        acc = None
        for rg in regions:
            h = 4 * rg + j
            lhs = lhs_ref[pl.ds(pl.multiple_of(h * 8, 8), 4), :].astype(_BF16)
            d = _dot(lhs, w_buf[rg, pl.ds(pl.multiple_of(j * 128, 128), 128), :])
            acc = d if acc is None else acc + d
        return acc

    z4 = jnp.zeros((4, 512), _F32)

    def f1(first):
        def body(a, ob_acc):
            for s in range(4):
                t = 4 * a + s
                pace(s_wob, [(None, s_woa)], t, 0)
                ev, od = head_pair(wuv_buf, a, s, 0, 8)
                for h, w in ((2 * t, ev), (2 * t + 1, od)):
                    row = pl.ds(pl.multiple_of(h * 8, 8), 4)
                    lhs = jnp.concatenate([cc_s[ct, row, :] for ct in range(4)], axis=1)
                    ctx_s[row, :] = _dot(lhs.astype(_BF16), w)
                pace(s_wob, [(None, s_woa)], t, 1)
                if not first:
                    ob_acc = ob_acc + proj(ob_s, wob_buf, a - 1, (2 * s, 2 * s + 1))
            return ob_acc
        return body
    f1(True)(0, z4)
    out_b = lax.fori_loop(1, 4, f1(False), z4)

    for s in range(4):
        pace(s_woa, [], s, 0)
        pace(s_woa, [], s, 1)
        out_b = out_b + proj(ob_s, wob_buf, 3, (2 * s, 2 * s + 1))
    out_ref[:, 512:] = out_b.astype(out_ref.dtype)

    def f2(t, acc):
        pace(s_woa, [], t, 0)
        pace(s_woa, [], t, 1)
        s = t % 4
        return acc + proj(ctx_s, woa_buf, t // 4 - 1, (2 * s, 2 * s + 1))
    out_a = lax.fori_loop(4, 16, f2, z4)
    out_a = out_a + proj(ctx_s, woa_buf, 3, range(8))
    out_ref[:, :512] = out_a.astype(out_ref.dtype)


@jax.jit
def pallas_concat_heads__compressed_kv_cla__gqa_block_cached__decode_kernel(A_x, A_c_kv, A_w_q, A_w_uk, A_w_uv, A_w_o, B_x, B_k_cache, B_v_cache, B_wq, B_wo):
    vm = pltpu.VMEM
    out = pl.pallas_call(
        _kernel,
        in_specs=[pl.BlockSpec(memory_space=pl.ANY)] * 11,
        out_specs=pl.BlockSpec(memory_space=pltpu.VMEM),
        out_shape=jax.ShapeDtypeStruct((4, 1024), _BF16),
        scratch_shapes=[
            vm((4, 512), _BF16), vm((4, 512), _BF16),
            vm((8, 2048, 128), _BF16), vm((8, 2048, 128), _BF16), vm((8, 2048, 128), _BF16),
            vm((8, 512, 512), _BF16), vm((8, 64, 4096), _BF16), vm((8, 512, 512), _BF16),
            vm((32, 4, 32, 512), _BF16), vm((8, 4096, 128), _BF16), vm((8, 4096, 128), _BF16),
            vm((32, 4, 128), _F32),
            vm((4, 256, 128), _F32),
            vm((4, 32, 512), _BF16),
            vm((256, 128), _F32),
            vm((4, 32, 128), _F32),
            vm((32, 32, 128), _F32),
            vm((32, 4, 8, 128), _F32),
            vm((256, 128), _F32),
            vm((4, 256, 128), _F32),
            vm((256, 128), _F32),
            pltpu.SemaphoreType.DMA((_LOOK * _MAXG,)),
            pltpu.SemaphoreType.DMA((_LOOK * _MAXG,)),
            pltpu.SemaphoreType.DMA((2,)),
        ],
        compiler_params=pltpu.CompilerParams(
            vmem_limit_bytes=64 * 1024 * 1024, disable_bounds_checks=True),
    )(
        A_x.reshape(4, 512), A_c_kv.reshape(4, 4, 1024, 512),
        A_w_q.reshape(8, 2048, 128), A_w_uk.reshape(8, 2048, 128), A_w_uv.reshape(8, 2048, 128),
        A_w_o.reshape(8, 512, 512),
        B_x.reshape(4, 512), B_k_cache, B_v_cache,
        B_wq.reshape(8, 64, 4096), B_wo.reshape(8, 512, 512),
    )
    return out.reshape(4, 1, 1024)
```

```python
import jax
import jax.numpy as jnp
from jax import lax
import jax.experimental.pallas as pl
import jax.experimental.pallas.tpu as pltpu

_NT = (((1,), (1,)), ((), ()))
_F32 = jnp.float32
_BF16 = jnp.bfloat16
_LOOK = 4
_MAXG = 3
CFG_KSHIFT = True
CFG_WSHIFT = True
_PITCH = 136


def _dot(a, b):
    return jnp.dot(a, b, preferred_element_type=_F32)


def _dot_nt(a, b):
    return lax.dot_general(a, b, _NT, preferred_element_type=_F32)


def _kernel(xa_hbm, c_hbm, wq_hbm, wuk_hbm, wuv_hbm, woa_hbm,
            xb_hbm, k_hbm, v_hbm, wqb_hbm, wob_hbm,
            out_ref,
            xa_buf, xb_buf, wq_buf, wuk_buf, wuv_buf, woa_buf, wqb_buf, wob_buf,
            c_buf, k_buf, v_buf,
            qa_s, qabs_s, qabs_t, qb_s, qb_t, sa_s, sb_s, ob_s, cc_s, rl_s, ctx_s,
            hsem, lsem, xsem):
    scale = 128 ** -0.5

    def sems(t, g):
        i = (t & (_LOOK - 1)) * _MAXG + g
        return hsem.at[i], lsem.at[i]

    def pair(src, dst, t, g):
        hs, ls = sems(t, g)
        hi = pltpu.make_async_copy(src(0, 1), dst(0, 1), hs)
        lo = pltpu.make_async_copy(src(1, 3), dst(1, 3), ls)
        return hi, lo

    def wait(t, g):
        view = lambda o, n: wq_buf.at[pl.ds(o, n), pl.ds(0, 128)]
        hi, lo = pair(view, view, t, g)
        lo.wait()
        hi.wait()

    def go(pairs):
        for hi, _ in pairs:
            hi.start(priority=0)
        for _, lo in pairs:
            lo.start(priority=1)

    class Stream:
        def __init__(self, steps, groups, fn, fn0=None):
            self.steps, self.groups, self.fn, self.fn0 = steps, groups, fn, fn0

        def start(self, t, g, early=False):
            if self.fn0 is None or g >= 2 or not early:
                go([self.fn(t, g)])
            elif isinstance(t, int):
                go(self.fn0(g) if t == 0 else [self.fn(t, g)])
            else:
                pl.when(t == 0)(lambda: go(self.fn0(g)))
                pl.when(t > 0)(lambda: go([self.fn(jnp.maximum(t, 1), g)]))

    def rows_pair(hbm, buf, src, dst, rows, t, g):
        r = pl.ds(src if isinstance(src, int) else pl.multiple_of(src, 8), rows)
        d = pl.ds(dst if isinstance(dst, int) else pl.multiple_of(dst, 8), rows)
        return pair(lambda o, n: hbm(g).at[pl.ds(o, n), r],
                    lambda o, n: buf(g).at[pl.ds(o, n), d], t, g)

    halves = lambda ref: (lambda g: ref.at[pl.ds(4 * g, 4)])
    parity = lambda ref: (lambda g: ref.at[:, g])

    def rows_fn(hbm, buf, rows):
        return lambda t, g: rows_pair(halves(hbm), halves(buf), t * rows, t * rows, rows, t, g)

    def gather_stream(hbm, buf):
        hbm, buf = halves(hbm), halves(buf)
        if not CFG_WSHIFT:
            return Stream(16, 2, lambda t, g: rows_pair(hbm, buf, t * 128, t * _PITCH, 128, t, g))
        return Stream(
            16, 2, lambda t, g: rows_pair(hbm, buf, t * 128 - 8, t * _PITCH, 128, t, g),
            lambda g: [rows_pair(hbm, buf, 0, 8, 120, 0, g),
                       rows_pair(hbm, buf, 2040, 16 * _PITCH, 8, 0, g)])

    def kv_fns(hbm, buf):
        hbm, buf = parity(hbm), parity(buf)
        if not CFG_KSHIFT:
            return (lambda t, g: rows_pair(hbm, buf, t * 128, t * 128, 128, t, g)), None
        return (lambda t, g: rows_pair(hbm, buf, t * 128 - 120, t * 128, 128, t, g),
                lambda g: [rows_pair(hbm, buf, 3976, 0, 120, 0, g),
                           rows_pair(hbm, buf, 0, 120, 8, 0, g)])

    def wqb_fn(t, g):
        r = pl.ds(pl.multiple_of((t >> 1) * 8, 8), 8)
        c = pl.ds(pl.multiple_of((t & 1) * 2048, 2048), 2048)
        return pair(lambda o, n: wqb_hbm.at[pl.ds(4 * g + o, n), r, c],
                    lambda o, n: wqb_buf.at[pl.ds(4 * g + o, n), r, c], t, g)

    def k_stream(b):
        kfn, kfn0 = kv_fns(k_hbm.at[b], k_buf)

        def fn(t, g):
            if g < 2:
                return kfn(t, g)
            r = pl.ds(pl.multiple_of(t * 32, 32), 32)
            return pair(lambda o, n: c_hbm.at[b, pl.ds(o, n), r],
                        lambda o, n: c_buf.at[t, pl.ds(o, n)], t, g)
        return Stream(32, 3, fn, kfn0)

    def v_stream(b):
        return Stream(32, 2, *kv_fns(v_hbm.at[b], v_buf))

    s_wq = gather_stream(wq_hbm, wq_buf)
    s_wuk = gather_stream(wuk_hbm, wuk_buf)
    s_wqb = Stream(16, 2, wqb_fn)
    s_wuv = gather_stream(wuv_hbm, wuv_buf)
    wo_hbm = lambda g: (wob_hbm, woa_hbm)[g]
    wo_buf = lambda g: (wob_buf, woa_buf)[g]
    s_wo = Stream(28, 2, lambda t, g: rows_pair(wo_hbm, wo_buf, t * 32, t * 32, 32, t, g))

    def wo_last_fn(t, g):
        view = lambda ref: (lambda o, n: ref.at[t, pl.ds(896 + 32 * o, 32 * n)])
        return pair(view(wo_hbm(g)), view(wo_buf(g)), t, g)
    s_wo_last = Stream(4, 2, wo_last_fn)

    def pace(cur, nxt, t, g):
        wait(t, g)

        @pl.when(t + _LOOK < cur.steps)
        def _():
            cur.start(t + _LOOK, g)

        for cond, st in nxt:
            gs = [g] if g < st.groups else []
            if g == cur.groups - 1:
                gs += list(range(cur.groups, st.groups))
            if not gs:
                continue
            c = t + _LOOK >= cur.steps
            if cond is not None:
                c = jnp.logical_and(c, cond)

            @pl.when(c)
            def _():
                for gg in gs:
                    st.start(t + _LOOK - cur.steps, gg, early=True)

    def head_pair(buf, a, s, lo, hi):
        wp = _PITCH // 2
        words = buf.bitcast(jnp.uint32)
        n = 15 * wp + 52
        if CFG_WSHIFT:
            view = words.at[:, pl.ds(pl.multiple_of(4 * a + 4, 4), n), :]
            last = words.at[:, pl.ds(pl.multiple_of(4 * a + 4 + 4 * ((a + 1) >> 2), 4), n), :]
        else:
            view = last = words.at[:, pl.ds(pl.multiple_of(4 * a, 4), n), :]
        x = jnp.concatenate(
            [(view if ml < 3 else last)[r, pl.ds(16 * ml + s, 16, stride=wp), :]
             for r in range(lo, hi) for ml in range(4)], axis=0)
        even = pltpu.bitcast(x << 16, _F32).astype(_BF16)
        odd = pltpu.bitcast(x & jnp.uint32(0xFFFF0000), _F32).astype(_BF16)
        return even, odd

    mi = lax.broadcasted_iota(jnp.int32, (128, 128), 0)
    ji = lax.broadcasted_iota(jnp.int32, (128, 128), 1)
    perm = jnp.where(mi == (ji & 64) + 4 * (ji & 15) + ((ji >> 4) & 3), 1.0, 0.0).astype(_BF16)

    for t in range(_LOOK):
        for g in range(2):
            s_wq.start(t, g, early=True)
    cxa = pltpu.make_async_copy(xa_hbm, xa_buf, xsem.at[0])
    cxb = pltpu.make_async_copy(xb_hbm, xb_buf, xsem.at[1])
    cxa.start()
    cxb.start()
    cxa.wait()
    cxb.wait()
    xa = jnp.concatenate(
        [_dot(xa_buf[:, 128 * k:128 * (k + 1)], perm) for k in range(4)], axis=1).astype(_BF16)
    xb = xb_buf[...]

    def p0(t, c):
        for g in range(2):
            pace(s_wq, [(None, s_wuk)], t, g)
        return c
    lax.fori_loop(0, 16, p0, 0)

    def p1(a, c):
        for s in range(4):
            t = 4 * a + s
            pace(s_wuk, [(None, s_wqb)], t, 0)
            ev, od = head_pair(wq_buf, a, s, 0, 8)
            qa_s[2 * t] = _dot(xa, ev)
            qa_s[2 * t + 1] = _dot(xa, od)
            pace(s_wuk, [(None, s_wqb)], t, 1)
        return c
    lax.fori_loop(0, 4, p1, 0)

    def p2(a, c):
        for s in range(4):
            t = 4 * a + s
            for g in range(2):
                pace(s_wqb, [(None, s_wuv)], t, g)
                ev, od = head_pair(wuk_buf, a, s, 4 * g, 4 * g + 4)
                for h, w in ((2 * t, ev), (2 * t + 1, od)):
                    r = _dot_nt(qa_s[h].astype(_BF16), w) * scale
                    row = pl.ds(pl.multiple_of(h * 8, 8), 4)
                    qabs_s[2 * g, row, :] = r[:, :128]
                    qabs_s[2 * g + 1, row, :] = r[:, 128:]
        return c
    lax.fori_loop(0, 4, p2, 0)

    nxt3 = [(None, k_stream(0))]
    pace(s_wuv, nxt3, 0, 0)
    for ct in range(4):
        r = jnp.concatenate(
            [qabs_s[ct, pl.ds(b, 32, stride=8), :] for b in range(4)], axis=0).astype(_BF16)
        qabs_t[:, 128 * ct:128 * (ct + 1)] = _dot_nt(r, perm).astype(_BF16)

    def p3(t, c):
        pace(s_wuv, nxt3, t, 1)
        w = wqb_buf[:, :, pl.ds(pl.multiple_of(t * 256, 256), 256)].reshape(512, 256)
        q = _dot(xb, w).astype(_BF16).astype(_F32) * scale
        qb_s[pl.ds(pl.multiple_of(t * 16, 8), 4), :] = q[:, :128]
        qb_s[pl.ds(pl.multiple_of(t * 16 + 8, 8), 4), :] = q[:, 128:]
        pace(s_wuv, nxt3, t + 1, 0)
        return c
    lax.fori_loop(0, 16, p3, 0)
    for b in range(4):
        qb_t[b] = qb_s[pl.ds(b, 32, stride=8), :]

    top = lax.broadcasted_iota(jnp.int32, (8, 128), 0) < 4

    def batch(b, carry):
        ks, vs = k_stream(b), v_stream(b)
        qb = [qb_t[b, 8 * i:8 * i + 8, :].astype(_BF16) for i in range(4)]
        qabs = qabs_t[pl.ds(pl.multiple_of(b * 32, 32), 32), :]

        def kstep(t, c):
            mb, ma = list(c[0]), c[1]
            r = pl.ds(pl.multiple_of(t * 128, 128), 128)
            pace(ks, [(None, vs)], t, 1)
            for i in range(4):
                s = jnp.where(top, _dot_nt(qb[i], k_buf[i, 0, r, :]),
                              _dot_nt(qb[i], k_buf[i, 1, r, :]))
                sb_s[t, i] = s
                mb[i] = jnp.maximum(mb[i], s)
            pace(ks, [(None, vs)], t, 2)
            sa = _dot_nt(qabs, c_buf[t].reshape(128, 512))
            sa_s[t] = sa
            pace(ks, [(None, vs)], t + 1, 0)
            return tuple(mb), jnp.maximum(ma, sa)

        ninf = lambda n: jnp.full((n, 128), -jnp.inf, _F32)
        mb, ma = lax.fori_loop(0, 32, kstep, ((ninf(8),) * 4, ninf(32)))
        mb = [jnp.broadcast_to(jnp.max(m, axis=-1, keepdims=True), (8, 128)) for m in mb]
        ma = jnp.broadcast_to(jnp.max(ma, axis=-1, keepdims=True), (32, 128))

        nxt = [(b < 3, k_stream(jnp.minimum(b + 1, 3))), (b == 3, s_wo)]

        def vstep(t, c):
            lb, ab, la, aa = list(c[0]), list(c[1]), c[2], c[3]
            r = pl.ds(pl.multiple_of(t * 128, 128), 128)
            pace(vs, nxt, t, 1)
            for i in range(4):
                p = jnp.exp(sb_s[t, i] - mb[i])
                lb[i] = lb[i] + p
                p = p.astype(_BF16)
                ab[i] = ab[i] + jnp.where(top, _dot(p, v_buf[i, 0, r, :]),
                                          _dot(p, v_buf[i, 1, r, :]))
            p = jnp.exp(sa_s[t] - ma)
            la = la + p
            aa = aa + _dot(p.astype(_BF16), c_buf[t].reshape(128, 512))
            pace(vs, nxt, t + 1, 0)
            return tuple(lb), tuple(ab), la, aa

        z8 = jnp.zeros((8, 128), _F32)
        lb, ab, la, aa = lax.fori_loop(
            0, 32, vstep,
            ((z8,) * 4, (z8,) * 4, jnp.zeros((32, 128), _F32), jnp.zeros((32, 512), _F32)))
        ob = jnp.concatenate(
            [ab[i] / jnp.sum(lb[i], axis=-1, keepdims=True) for i in range(4)], axis=0)
        rl = jnp.broadcast_to(1.0 / jnp.sum(la, axis=-1, keepdims=True), (32, 128))
        aa = aa.astype(_BF16)
        cc = [_dot(aa[:, 128 * ct:128 * (ct + 1)], perm) for ct in range(4)]
        for bb in range(4):
            @pl.when(b == bb)
            def _():
                rows = pl.ds(bb, 32, stride=8)
                ob_s[rows, :] = ob
                rl_s[rows, :] = rl
                for ct in range(4):
                    cc_s[ct, rows, :] = cc[ct]
        return carry
    lax.fori_loop(0, 4, batch, 0)

    def proj(lhs_ref, w_buf, rg, j):
        h = 8 * rg + j
        lhs = lhs_ref[pl.ds(pl.multiple_of(h * 8, 8), 4), :].astype(_BF16)
        return _dot(lhs, w_buf[rg, pl.ds(pl.multiple_of(j * 128, 128), 128), :])

    nxtf = [(None, s_wo_last)]

    def fstep(s):
        def body(t, acc):
            out_a, out_b = acc
            rg, j = t & 3, (t >> 2) - 1
            if s != 0:
                out_b = out_b + proj(ob_s, wob_buf, rg, j)
                out_a = out_a + proj(ctx_s, woa_buf, rg, j)
            pace(s_wo, nxtf, t, 1)
            if s is not None:
                ev, od = head_pair(wuv_buf, rg, s, 0, 8)
                for h, w in ((8 * rg + 2 * s, ev), (8 * rg + 2 * s + 1, od)):
                    row = pl.ds(pl.multiple_of(h * 8, 8), 4)
                    lhs = jnp.concatenate([cc_s[ct, row, :] for ct in range(4)], axis=1)
                    ctx_s[row, :] = _dot(lhs.astype(_BF16), w) * rl_s[row, :]
            wait(t + 1, 0)

            @pl.when(t + 1 + _LOOK < s_wo.steps)
            def _():
                s_wo.start(t + 1 + _LOOK, 0)

            @pl.when(jnp.logical_and(t + 1 + _LOOK >= s_wo.steps, t + 1 < s_wo.steps))
            def _():
                s_wo_last.start(t + 1 + _LOOK - s_wo.steps, 0)
            return out_a, out_b
        return body

    z4 = jnp.zeros((4, 512), _F32)
    acc = (z4, z4)
    for s in range(4):
        acc = lax.fori_loop(8 * s, 8 * s + 4, fstep(s), acc)
        if s < 3:
            acc = lax.fori_loop(8 * s + 4, 8 * s + 8, fstep(None), acc)
    out = list(acc[::-1])
    lhs_of, w_of = (ob_s, ctx_s), (wob_buf, woa_buf)
    for rg in range(4):
        for g in range(2):
            out[g] = out[g] + proj(lhs_of[g], w_of[g], rg, 6)
    for u in range(8):
        rg, g = u >> 1, u & 1
        if u in (1, 5, 7):
            for v in range(u, {1: 5, 5: 7, 7: 8}[u]):
                wait(v >> 1, v & 1)
        out[g] = out[g] + proj(lhs_of[g], w_of[g], rg, 7)
        if u == 6:
            out_ref[:, 512:] = out[0].astype(out_ref.dtype)
    out_ref[:, :512] = out[1].astype(out_ref.dtype)


@jax.jit
def pallas_concat_heads__compressed_kv_cla__gqa_block_cached__decode_kernel(A_x, A_c_kv, A_w_q, A_w_uk, A_w_uv, A_w_o, B_x, B_k_cache, B_v_cache, B_wq, B_wo):
    vm = pltpu.VMEM
    out = pl.pallas_call(
        _kernel,
        in_specs=[pl.BlockSpec(memory_space=pl.ANY)] * 11,
        out_specs=pl.BlockSpec(memory_space=pltpu.VMEM),
        out_shape=jax.ShapeDtypeStruct((4, 1024), _BF16),
        scratch_shapes=[
            vm((4, 512), _BF16), vm((4, 512), _BF16),
            vm((8, 16 * _PITCH + 8, 128), _BF16), vm((8, 16 * _PITCH + 8, 128), _BF16),
            vm((8, 16 * _PITCH + 8, 128), _BF16),
            vm((4, 1024, 512), _BF16), vm((8, 64, 4096), _BF16), vm((4, 1024, 512), _BF16),
            vm((32, 4, 32, 512), _BF16), vm((4, 2, 4096, 128), _BF16), vm((4, 2, 4096, 128), _BF16),
            vm((32, 4, 128), _F32),
            vm((4, 256, 128), _F32),
            vm((128, 512), _BF16),
            vm((256, 128), _F32),
            vm((4, 32, 128), _F32),
            vm((32, 32, 128), _F32),
            vm((32, 4, 8, 128), _F32),
            vm((256, 128), _F32),
            vm((4, 256, 128), _F32),
            vm((256, 128), _F32),
            vm((256, 128), _F32),
            pltpu.SemaphoreType.DMA((_LOOK * _MAXG,)),
            pltpu.SemaphoreType.DMA((_LOOK * _MAXG,)),
            pltpu.SemaphoreType.DMA((2,)),
        ],
        compiler_params=pltpu.CompilerParams(
            vmem_limit_bytes=64 * 1024 * 1024, disable_bounds_checks=True,
            disable_semaphore_checks=True),
    )(
        A_x.reshape(4, 512), A_c_kv.reshape(4, 4, 1024, 512),
        A_w_q.reshape(8, 2048, 128), A_w_uk.reshape(8, 2048, 128), A_w_uv.reshape(8, 2048, 128),
        A_w_o.reshape(4, 1024, 512),
        B_x.reshape(4, 512), B_k_cache.reshape(4, 4, 2, 4096, 128),
        B_v_cache.reshape(4, 4, 2, 4096, 128),
        B_wq.reshape(8, 64, 4096), B_wo.reshape(4, 1024, 512),
    )
    return out.reshape(4, 1, 1024)
```

```python
import jax
import jax.numpy as jnp
from jax import lax
import jax.experimental.pallas as pl
import jax.experimental.pallas.tpu as pltpu

_NT = (((1,), (1,)), ((), ()))
_F32 = jnp.float32
_BF16 = jnp.bfloat16
_LOOK = 4
_PITCH = 136
CFG_CALIGN = True


def _dot(a, b):
    return jnp.dot(a, b, preferred_element_type=_F32)


def _dot_nt(a, b):
    return lax.dot_general(a, b, _NT, preferred_element_type=_F32)


def _ds(start, size, mult=8):
    if not isinstance(start, int):
        start = pl.multiple_of(start, mult)
    return pl.ds(start, size)


def _kernel(xa_hbm, c_hbm, wq_hbm, wuk_hbm, wuv_hbm, woa_hbm,
            xb_hbm, k_hbm, v_hbm, wqb_hbm, wob_hbm,
            out_ref,
            xa_buf, xb_buf, wq_buf, wuk_buf, wuv_buf, woa_buf, wqb_buf, wob_buf,
            c_buf, k_buf, v_buf,
            perm_s, qa_s, qabs_s, qabs_t, qb_s, qb_t, sa_s, ma_s, sb_s, ob_s, cc_s, rl_s, ctx_s,
            hsem, lsem, xsem):
    scale = 128 ** -0.5

    def pair(src, dst, t, g):
        i = (t & (_LOOK - 1)) * 2 + g
        hi = pltpu.make_async_copy(src(3, 1), dst(3, 1), hsem.at[i])
        lo = pltpu.make_async_copy(src(0, 3), dst(0, 3), lsem.at[i])
        return hi, lo

    def wait(t, g):
        view = lambda o, n: k_buf.at[pl.ds(o, n), 0, pl.ds(0, 128)]
        hi, lo = pair(view, view, t, g)
        lo.wait()
        hi.wait()

    def go(pairs):
        for hi, _ in pairs:
            hi.start(priority=0)
        for _, lo in pairs:
            lo.start(priority=1)

    class Stream:
        def __init__(self, steps, fn, fn0=None):
            self.steps, self.fn, self.fn0 = steps, fn, fn0

        def start(self, t, g, early=False):
            if self.fn0 is None or not early:
                go(self.fn(t, g))
            else:
                pl.when(t == 0)(lambda: go(self.fn0(g)))
                pl.when(t > 0)(lambda: go(self.fn(jnp.maximum(t, 1), g)))

    def box(hbm, buf, src, dst, t, g):
        return pair(lambda o, n: hbm.at[(pl.ds(o, n),) + src],
                    lambda o, n: buf.at[(pl.ds(o, n),) + dst], t, g)

    def gather_stream(hbm, buf):
        def rows(src, dst, n, t, g):
            return box(hbm.at[g], buf.at[g], (_ds(src, n),), (_ds(dst, n),), t, g)
        return Stream(16, lambda t, g: [rows(t * 128 - 8, t * _PITCH, 128, t, g)],
                      lambda g: [rows(0, 8, 120, 0, g), rows(2040, 16 * _PITCH, 8, 0, g)])

    def kv_stream(hbm, buf):
        def rows(src, dst, n, t, g):
            return box(hbm, buf, (g, _ds(src, n)), (g, _ds(dst, n)), t, g)
        return Stream(32, lambda t, g: [rows(t * 128 - 120, t * 128, 128, t, g)],
                      lambda g: [rows(3976, 0, 120, 0, g), rows(0, 120, 8, 0, g)])

    def wqb_fn(t, g):
        idx = (_ds((t >> 1) * 8, 8), _ds((t & 1) * 2048, 2048, 2048))
        return [box(wqb_hbm.at[g], wqb_buf.at[g], idx, idx, t, g)]

    def c_fn(t, g):
        hbm = c_hbm.at[t >> 5]
        r = (t & 31) * 32
        if not CFG_CALIGN:
            return [box(hbm, c_buf.at[t], (g, _ds(r, 32)), (g,), t, g)]
        tp = (t + 31) & 31
        tail, head = pl.ds(384, 128), pl.ds(0, 384)
        return [box(hbm, c_buf.at[(t & 32) + tp], (g, _ds(tp * 32 + 24, 8), tail),
                    (g, pl.ds(24, 8), tail), t, g),
                box(hbm, c_buf.at[t], (g, _ds(r, 24)), (g, pl.ds(0, 24)), t, g),
                box(hbm, c_buf.at[t], (g, _ds(r + 24, 8), head), (g, pl.ds(24, 8), head), t, g)]

    wo_hbm, wo_buf = (wob_hbm, woa_hbm), (wob_buf, woa_buf)

    def wo_fn(t, g):
        idx = (_ds(t * 32, 32),)
        return [box(wo_hbm[g], wo_buf[g], idx, idx, t, g)]

    def wo_last_fn(t, g):
        view = lambda ref: (lambda o, n: ref.at[t, pl.ds(896 + 32 * o, 32 * n)])
        return [pair(view(wo_hbm[g]), view(wo_buf[g]), t, g)]

    s_wq = gather_stream(wq_hbm, wq_buf)
    s_wuk = gather_stream(wuk_hbm, wuk_buf)
    s_wqb = Stream(16, wqb_fn)
    s_wuv = gather_stream(wuv_hbm, wuv_buf)
    s_c = Stream(64, c_fn)
    k_stream = lambda b: kv_stream(k_hbm.at[b], k_buf)
    v_stream = lambda b: kv_stream(v_hbm.at[b], v_buf)
    s_wo = Stream(28, wo_fn)
    s_wo_last = Stream(4, wo_last_fn)

    def issue(cur, nxt, t, g, skip0=False):
        c = t + _LOOK < cur.steps
        if skip0:
            c = jnp.logical_and(c, t > 0)
        pl.when(c)(lambda: cur.start(t + _LOOK, g))
        for cond, st in nxt:
            c = jnp.logical_and(t + _LOOK >= cur.steps, t + _LOOK - cur.steps < st.steps)
            if cond is not None:
                c = jnp.logical_and(c, cond)
            pl.when(c)(lambda st=st: st.start(t + _LOOK - cur.steps, g, early=True))

    def pace(cur, nxt, t, g):
        wait(t, g)
        issue(cur, nxt, t, g)

    def head_pair(buf, a, s, lo, hi):
        wp = _PITCH // 2
        words = buf.bitcast(jnp.uint32)
        n = 15 * wp + 52
        view = words.at[:, :, _ds(4 * a + 4, n, 4), :]
        last = words.at[:, :, _ds(4 * a + 4 + 4 * ((a + 1) >> 2), n, 4), :]
        x = jnp.concatenate(
            [(view if ml < 3 else last)[r // 4, r % 4, pl.ds(16 * ml + s, 16, stride=wp), :]
             for r in range(lo, hi) for ml in range(4)], axis=0)
        even = pltpu.bitcast(x << 16, _F32).astype(_BF16)
        odd = pltpu.bitcast(x & jnp.uint32(0xFFFF0000), _F32).astype(_BF16)
        return even, odd

    units = [s_wq.fn0(g) if t == 0 else s_wq.fn(t, g) for t in range(_LOOK) for g in range(2)]
    for hi, _ in units[0]:
        hi.start(priority=0)
    for u in units:
        for _, lo in u:
            lo.start(priority=1)
    cxa = pltpu.make_async_copy(xa_hbm, xa_buf, xsem.at[0])
    cxb = pltpu.make_async_copy(xb_hbm, xb_buf, xsem.at[1])
    cxa.start()
    cxb.start()

    ji = lax.broadcasted_iota(jnp.int32, (1, 128), 1)
    src_row = (ji & 64) + 4 * (ji & 15) + ((ji >> 4) & 3)

    def perm_row(m, c):
        perm_s[pl.ds(m, 1), :] = jnp.where(src_row == m, 1.0, 0.0)
        return c
    for k in range(8):
        lax.fori_loop(16 * k, 16 * k + 16, perm_row, 0)
        if k < 7:
            for hi, _ in units[k + 1]:
                hi.start(priority=0)

    def p0(t, c):
        for g in range(2):
            pace(s_wq, [(None, s_wuk)], t, g)
        return c
    lax.fori_loop(0, 16, p0, 0)
    cxa.wait()
    cxb.wait()
    perm = perm_s[...].astype(_BF16)
    xa = jnp.concatenate(
        [_dot(xa_buf[:, 128 * k:128 * (k + 1)], perm) for k in range(4)], axis=1).astype(_BF16)
    xb = xb_buf[...]
    ma_s[...] = jnp.full(ma_s.shape, -jnp.inf, _F32)

    def p1(a, c):
        for s in range(4):
            t = 4 * a + s
            pace(s_wuk, [(None, s_wqb)], t, 0)
            ev, od = head_pair(wq_buf, a, s, 0, 8)
            qa_s[2 * t] = _dot(xa, ev)
            qa_s[2 * t + 1] = _dot(xa, od)
            pace(s_wuk, [(None, s_wqb)], t, 1)
        return c
    lax.fori_loop(0, 4, p1, 0)

    def p2(a, c):
        for s in range(4):
            t = 4 * a + s
            for g in range(2):
                pace(s_wqb, [(None, s_wuv)], t, g)
                ev, od = head_pair(wuk_buf, a, s, 4 * g, 4 * g + 4)
                for h, w in ((2 * t, ev), (2 * t + 1, od)):
                    r = _dot_nt(qa_s[h].astype(_BF16), w) * scale
                    qabs_s[2 * g, _ds(h * 8, 4), :] = r[:, :128]
                    qabs_s[2 * g + 1, _ds(h * 8, 4), :] = r[:, 128:]
        return c
    lax.fori_loop(0, 4, p2, 0)

    nxt = [(None, s_c)]
    pace(s_wuv, nxt, 0, 0)
    for ct in range(4):
        r = jnp.concatenate(
            [qabs_s[ct, pl.ds(b, 32, stride=8), :] for b in range(4)], axis=0).astype(_BF16)
        qabs_t[:, 128 * ct:128 * (ct + 1)] = _dot_nt(r, perm).astype(_BF16)

    def p3(t, c):
        pace(s_wuv, nxt, t, 1)
        w = wqb_buf[:, :, :, _ds(t * 256, 256, 256)].reshape(512, 256)
        q = _dot(xb, w).astype(_BF16).astype(_F32) * scale
        qb_s[_ds(t * 16, 4), :] = q[:, :128]
        qb_s[_ds(t * 16 + 8, 4), :] = q[:, 128:]
        pace(s_wuv, nxt, t + 1, 0)
        return c
    lax.fori_loop(0, 16, p3, 0)
    for b in range(4):
        qb_t[b] = qb_s[pl.ds(b, 32, stride=8), :]

    nxt = [(None, k_stream(0))]

    def c_block(t, jb):
        return c_buf[t, pl.ds(2 * jb, 2)].reshape(128, 512)

    def c_scores(t, jb):
        b = 2 * (t >> 5) + jb
        sa = _dot_nt(qabs_t[_ds(b * 32, 32, 32), :], c_block(t, jb))
        sa_s[t, jb] = sa
        ma_s[b] = jnp.maximum(ma_s[b], sa)

    pace(s_c, nxt, 0, 1)
    pace(s_c, nxt, 1, 0)

    def cstep(t, c):
        wait(t, 1)
        c_scores(t - 1, 0)
        issue(s_c, nxt, t, 1)
        wait(t + 1, 0)
        c_scores(t - 1, 1)
        issue(s_c, nxt, t + 1, 0)
        return c
    lax.fori_loop(1, 64, cstep, 0)
    c_scores(63, 0)
    c_scores(63, 1)

    top = lax.broadcasted_iota(jnp.int32, (8, 128), 0) < 4

    def batch(b, carry):
        ks, vs = k_stream(b), v_stream(b)
        qb = [qb_t[b, 8 * i:8 * i + 8, :].astype(_BF16) for i in range(4)]

        def kstep(t, mb):
            mb = list(mb)
            r = _ds(t * 128, 128, 128)
            se = [_dot_nt(qb[i], k_buf[i, 0, r, :]) for i in range(4)]
            issue(ks, [(None, vs)], t, 0, skip0=True)
            wait(t, 1)
            for i in range(4):
                s = jnp.where(top, se[i], _dot_nt(qb[i], k_buf[i, 1, r, :]))
                sb_s[t, i] = s
                mb[i] = jnp.maximum(mb[i], s)
            issue(ks, [(None, vs)], t, 1)
            wait(t + 1, 0)
            return tuple(mb)

        mb = lax.fori_loop(0, 32, kstep, (jnp.full((8, 128), -jnp.inf, _F32),) * 4)
        vs.start(_LOOK, 0)
        mb = [jnp.broadcast_to(jnp.max(m, axis=-1, keepdims=True), (8, 128)) for m in mb]
        ma = jnp.broadcast_to(jnp.max(ma_s[b], axis=-1, keepdims=True), (32, 128))

        nxt = [(b < 3, k_stream(jnp.minimum(b + 1, 3))), (b == 3, s_wo)]

        def vstep(t, c):
            lb, ab, la, aa = list(c[0]), list(c[1]), c[2], c[3]
            r = _ds(t * 128, 128, 128)
            issue(vs, nxt, t, 0, skip0=True)
            tc = (b >> 1) * 32 + t
            p = jnp.exp(sa_s[tc, b & 1] - ma)
            la = la + p
            aa = aa + _dot(p.astype(_BF16), c_block(tc, b & 1))
            wait(t, 1)
            for i in range(4):
                p = jnp.exp(sb_s[t, i] - mb[i])
                lb[i] = lb[i] + p
                p = p.astype(_BF16)
                ab[i] = ab[i] + jnp.where(top, _dot(p, v_buf[i, 0, r, :]),
                                          _dot(p, v_buf[i, 1, r, :]))
            issue(vs, nxt, t, 1)
            wait(t + 1, 0)
            return tuple(lb), tuple(ab), la, aa

        z8 = jnp.zeros((8, 128), _F32)
        lb, ab, la, aa = lax.fori_loop(
            0, 32, vstep,
            ((z8,) * 4, (z8,) * 4, jnp.zeros((32, 128), _F32), jnp.zeros((32, 512), _F32)))
        for cond, st in nxt:
            pl.when(cond)(lambda st=st: st.start(_LOOK, 0))
        ob = jnp.concatenate(
            [ab[i] / jnp.sum(lb[i], axis=-1, keepdims=True) for i in range(4)], axis=0)
        rl = jnp.broadcast_to(1.0 / jnp.sum(la, axis=-1, keepdims=True), (32, 128))
        aa = aa.astype(_BF16)
        cc = [_dot(aa[:, 128 * ct:128 * (ct + 1)], perm) for ct in range(4)]
        for bb in range(4):
            @pl.when(b == bb)
            def _():
                rows = pl.ds(bb, 32, stride=8)
                ob_s[rows, :] = ob
                rl_s[rows, :] = rl
                for ct in range(4):
                    cc_s[ct, rows, :] = cc[ct]
        return carry
    lax.fori_loop(0, 4, batch, 0)

    lhs_of = (ob_s, ctx_s)

    def proj(g, rg, j):
        lhs = lhs_of[g][_ds((8 * rg + j) * 8, 4), :].astype(_BF16)
        return _dot(lhs, wo_buf[g][rg, _ds(j * 128, 128, 128), :])

    nxt = [(None, s_wo_last)]

    def fstep(s):
        def body(t, out):
            rg, j = t & 3, (t >> 2) - 1
            if s != 0:
                out = tuple(out[g] + proj(g, rg, j) for g in range(2))
            pace(s_wo, nxt, t, 1)
            if s is not None:
                ev, od = head_pair(wuv_buf, rg, s, 0, 8)
                for h, w in ((8 * rg + 2 * s, ev), (8 * rg + 2 * s + 1, od)):
                    row = _ds(h * 8, 4)
                    lhs = jnp.concatenate([cc_s[ct, row, :] for ct in range(4)], axis=1)
                    ctx_s[row, :] = _dot(lhs.astype(_BF16), w) * rl_s[row, :]
            pace(s_wo, nxt, t + 1, 0)
            return out
        return body

    acc = (jnp.zeros((4, 512), _F32),) * 2
    for s in range(4):
        acc = lax.fori_loop(8 * s, 8 * s + 4, fstep(s), acc)
        if s < 3:
            acc = lax.fori_loop(8 * s + 4, 8 * s + 8, fstep(None), acc)
    out = list(acc)
    for rg in range(4):
        for g in range(2):
            out[g] = out[g] + proj(g, rg, 6)
    for u in range(8):
        rg, g = u >> 1, u & 1
        if u in (1, 5, 7):
            for v in range(u, {1: 5, 5: 7, 7: 8}[u]):
                wait(v >> 1, v & 1)
        out[g] = out[g] + proj(g, rg, 7)
        if u == 6:
            out_ref[:, 512:] = out[0].astype(out_ref.dtype)
    out_ref[:, :512] = out[1].astype(out_ref.dtype)


@jax.jit
def pallas_concat_heads__compressed_kv_cla__gqa_block_cached__decode_kernel(A_x, A_c_kv, A_w_q, A_w_uk, A_w_uv, A_w_o, B_x, B_k_cache, B_v_cache, B_wq, B_wo):
    vm = pltpu.VMEM
    gather_buf = vm((2, 4, 16 * _PITCH + 8, 128), _BF16)
    out = pl.pallas_call(
        _kernel,
        in_specs=[pl.BlockSpec(memory_space=pl.ANY)] * 11,
        out_specs=pl.BlockSpec(memory_space=pltpu.VMEM),
        out_shape=jax.ShapeDtypeStruct((4, 1024), _BF16),
        scratch_shapes=[
            vm((4, 512), _BF16), vm((4, 512), _BF16),
            gather_buf, gather_buf, gather_buf,
            vm((4, 1024, 512), _BF16), vm((2, 4, 64, 4096), _BF16), vm((4, 1024, 512), _BF16),
            vm((64, 4, 2, 32, 512), _BF16),
            vm((4, 2, 4096, 128), _BF16), vm((4, 2, 4096, 128), _BF16),
            vm((128, 128), _F32),
            vm((32, 4, 128), _F32),
            vm((4, 256, 128), _F32),
            vm((128, 512), _BF16),
            vm((256, 128), _F32),
            vm((4, 32, 128), _F32),
            vm((64, 2, 32, 128), _F32),
            vm((4, 32, 128), _F32),
            vm((32, 4, 8, 128), _F32),
            vm((256, 128), _F32),
            vm((4, 256, 128), _F32),
            vm((256, 128), _F32),
            vm((256, 128), _F32),
            pltpu.SemaphoreType.DMA((_LOOK * 2,)),
            pltpu.SemaphoreType.DMA((_LOOK * 2,)),
            pltpu.SemaphoreType.DMA((2,)),
        ],
        compiler_params=pltpu.CompilerParams(
            vmem_limit_bytes=80 * 1024 * 1024, disable_bounds_checks=True,
            disable_semaphore_checks=True),
    )(
        A_x.reshape(4, 512), A_c_kv.reshape(2, 4, 2, 1024, 512),
        A_w_q.reshape(2, 4, 2048, 128), A_w_uk.reshape(2, 4, 2048, 128),
        A_w_uv.reshape(2, 4, 2048, 128), A_w_o.reshape(4, 1024, 512),
        B_x.reshape(4, 512), B_k_cache.reshape(4, 4, 2, 4096, 128),
        B_v_cache.reshape(4, 4, 2, 4096, 128),
        B_wq.reshape(2, 4, 64, 4096), B_wo.reshape(4, 1024, 512),
    )
    return out.reshape(4, 1, 1024)
```

```python
import jax
import jax.numpy as jnp
from jax import lax
import jax.experimental.pallas as pl
import jax.experimental.pallas.tpu as pltpu

_F32 = jnp.float32
_BF16 = jnp.bfloat16
_LOOK = 4
_PITCH = 136


def _dot(a, b):
    return jnp.dot(a, b, preferred_element_type=_F32)


def _dot_nt(a, b):
    return lax.dot_general(a, b, (((1,), (1,)), ((), ())), preferred_element_type=_F32)


def _ds(start, size, mult=8):
    if not isinstance(start, int):
        start = pl.multiple_of(start, mult)
    return pl.ds(start, size)


def _when(*conds):
    if any(c is False for c in conds):
        return lambda f: None
    traced = [c for c in conds if c is not True]
    if not traced:
        return lambda f: f()
    cond = traced[0]
    for c in traced[1:]:
        cond = jnp.logical_and(cond, c)
    return pl.when(cond)


def _kernel(xa_hbm, c_hbm, wq_hbm, wuk_hbm, wuv_hbm, woa_hbm,
            xb_hbm, k_hbm, v_hbm, wqb_hbm, wob_hbm,
            out_ref,
            xa_buf, xb_buf, wq_buf, wuk_buf, wuv_buf, woa_buf, wqb_buf, wob_buf,
            c_buf, k_buf, v_buf, size_ref,
            perm_s, qa_s, qabs_s, qabs_t, qb_s, qb_t, sa_s, ma_s, sb_s, ob_s, cc_s, rl_s, ctx_s,
            hsem, lsem, xsem):
    scale = 128 ** -0.5

    def copies(unit, t, g):
        i = (t & (_LOOK - 1)) * 2 + g
        return ([pltpu.make_async_copy(a, b, hsem.at[i]) for a, b in unit[0]],
                [pltpu.make_async_copy(a, b, lsem.at[i]) for a, b in unit[1]])

    def wait(t, g):
        hi, lo = size_ref.at[pl.ds(0, 1)], size_ref.at[pl.ds(0, 3)]
        hi, lo = copies(([(hi, hi)], [(lo, lo)]), t, g)
        lo[0].wait()
        hi[0].wait()

    def go(unit, t, g):
        his, los = copies(unit, t, g)
        for c in his:
            c.start(priority=0)
        for c in los:
            c.start(priority=1)

    class Stream:
        def __init__(self, steps, fn, wraps=lambda g: False):
            self.steps, self.fn, self.wraps = steps, fn, wraps

        def start(self, t, g, maybe0=False):
            if maybe0 and self.wraps(g) and not isinstance(t, int):
                pl.when(t == 0)(lambda: go(self.fn(0, g), 0, g))
                pl.when(t > 0)(lambda: go(self.fn(jnp.maximum(t, 1), g), t, g))
            else:
                go(self.fn(t, g), t, g)

    def views(hbm, buf, lead, boxes):
        return [(hbm.at[lead + a], buf.at[lead + b]) for a, b in boxes]

    def row_piece(hbm, buf, rows, rows0):
        def piece(lead, p):
            rs = rows0 if isinstance(p, int) and p == 0 else [rows(p)]
            return views(hbm, buf, lead, [((_ds(a, n),), (_ds(b, n),)) for a, b, n in rs])
        return piece

    def gather_piece(hbm, buf):
        return row_piece(hbm, buf, lambda p: (p * 128 - 8, p * _PITCH, 128),
                         [(0, 8, 120), (4088, 32 * _PITCH, 8)])

    def kv_piece(hbm, buf):
        return row_piece(hbm, buf, lambda p: (p * 128 - 120, p * 128, 128),
                         [(3976, 0, 120), (0, 120, 8)])

    def wqb_piece(lead, p):
        h = p & 1
        boxes = [(_ds((p >> 1) * 8, 8), _ds(h * 2048 + 128, 1920, 128)),
                 (_ds((((p + 1) >> 1) & 7) * 8, 8), _ds((1 - h) * 2048, 128, 128))]
        return views(wqb_hbm, wqb_buf, lead, [(x, x) for x in boxes])

    def c_piece(lead, p):
        hbm, r, q = c_hbm.at[p >> 5], (p & 31) * 32, (p + 31) & 31
        tail, head = pl.ds(384, 128), pl.ds(0, 384)
        return (views(hbm, c_buf.at[(p & 32) + q], lead,
                      [((_ds(q * 32 + 24, 8), tail), (pl.ds(24, 8), tail))])
                + views(hbm, c_buf.at[p], lead,
                        [((_ds(r, 24),), (pl.ds(0, 24),)),
                         ((_ds(r + 24, 8), head), (pl.ds(24, 8), head))]))

    def woa_piece(lead, p):
        boxes = [(_ds(jnp.where(p == 0, 888, p * 32 - 8), 8), pl.ds(384, 128)),
                 (_ds(p * 32, 24),), (_ds(p * 32 + 24, 8), pl.ds(0, 384))]
        return views(woa_hbm, woa_buf, lead, [(x, x) for x in boxes])

    def wob_piece(lead, p):
        boxes = [(_ds(p * 32, 8), pl.ds(128, 384)), (_ds(p * 32 + 8, 24),),
                 (_ds(jnp.where(p == 27, 0, p * 32 + 32), 8), pl.ds(0, 128))]
        return views(wob_hbm, wob_buf, lead, [(x, x) for x in boxes])

    def quad(piece, p, pre=(), post=()):
        return piece(pre + (pl.ds(3, 1),) + post, p), piece(pre + (pl.ds(0, 3),) + post, p)

    def cross(px, py):
        def fn(t, g):
            x, y = (px, py) if g == 0 else (py, px)
            return y((pl.ds(1, 1), g), t), x((pl.ds(0, 2), g), t) + y((pl.ds(0, 1), g), t)
        return fn

    wo_hbm, wo_buf = (wob_hbm, woa_hbm), (wob_buf, woa_buf)

    def wo_last(t, g):
        rows = lambda a, n: views(wo_hbm[g], wo_buf[g], (t >> 1, t & 1), [((pl.ds(a, n),),) * 2])
        return rows(992, 32), rows(896, 96)

    always = lambda g: True
    s_wa = Stream(32, cross(gather_piece(wuk_hbm, wuk_buf), gather_piece(wq_hbm, wq_buf)), always)
    s_wqb = Stream(16, lambda t, g: quad(wqb_piece, t, pre=(g,)))
    s_wuv = Stream(16, lambda t, g: quad(gather_piece(wuv_hbm, wuv_buf), t + 16 * g),
                   lambda g: g == 0)
    s_c = Stream(64, lambda t, g: quad(c_piece, t, post=(g,)))
    k_stream = lambda b: Stream(
        32, lambda t, g: quad(kv_piece(k_hbm.at[b], k_buf), t, post=(g,)), always)
    v_stream = lambda b: Stream(
        32, lambda t, g: quad(kv_piece(v_hbm.at[b], v_buf), t, post=(g,)), always)
    s_wo = Stream(28, cross(wob_piece, woa_piece))
    s_wo_last = Stream(4, wo_last)

    def issue(cur, nxt, t, g, skip0=False):
        u = t + _LOOK
        _when(u < cur.steps, t > 0 if skip0 else True)(lambda: cur.start(u, g))
        for cond, st in nxt:
            _when(u >= cur.steps, cond)(lambda st=st: st.start(u - cur.steps, g, maybe0=True))

    def pace(cur, nxt, t, g):
        wait(t, g)
        issue(cur, nxt, t, g)

    def head_pair(buf, a, s, lo, hi):
        wp = _PITCH // 2
        lead = (slice(None),) * (len(buf.shape) - 2)
        reg = (lambda r: (r,)) if len(lead) == 1 else (lambda r: (r // 2, r % 2))
        words = buf.bitcast(jnp.uint32)
        n = 31 * wp + 52
        view = words.at[lead + (_ds(4 * a + 4, n, 4),)]
        last = words.at[lead + (_ds(4 * a + 4 + 4 * ((a + 1) >> 2), n, 4),)]
        x = jnp.concatenate(
            [(view if ml < 3 else last)[reg(r) + (pl.ds(16 * ml + s, 32, stride=wp), slice(None))]
             for r in range(lo, hi) for ml in range(4)], axis=0)
        even = pltpu.bitcast(x << 16, _F32).astype(_BF16)
        odd = pltpu.bitcast(x & jnp.uint32(0xFFFF0000), _F32).astype(_BF16)
        return even, odd

    units = [copies(s_wa.fn(t, g), t, g) for t in range(_LOOK) for g in range(2)]
    for c in units[0][0]:
        c.start(priority=0)
    for _, los in units:
        for c in los:
            c.start(priority=1)
    cxa = pltpu.make_async_copy(xa_hbm, xa_buf, xsem.at[0])
    cxb = pltpu.make_async_copy(xb_hbm, xb_buf, xsem.at[1])
    cxa.start()
    cxb.start()

    ji = lax.broadcasted_iota(jnp.int32, (1, 128), 1)
    src_row = 4 * (ji & 31) + (ji >> 5)

    def perm_row(m, c):
        perm_s[pl.ds(m, 1), :] = jnp.where(src_row == m, 1.0, 0.0)
        return c
    for k in range(8):
        lax.fori_loop(16 * k, 16 * k + 16, perm_row, 0)
        if k < 7:
            for c in units[k + 1][0]:
                c.start(priority=0)

    def clear(row):
        wq_buf[:, :, _ds(row, 8), :] = jnp.zeros((2, 2, 8, 128), _BF16)
        wuk_buf[:, :, _ds(row, 8), :] = jnp.zeros((2, 2, 8, 128), _BF16)
        wuv_buf[:, _ds(row, 8), :] = jnp.zeros((4, 8, 128), _BF16)

    def pa(t, c):
        for g in range(2):
            pace(s_wa, [(True, s_wqb)], t, g)
        clear(jnp.maximum(t * _PITCH - 8, 0))
        return c
    lax.fori_loop(0, 32, pa, 0)
    clear(32 * _PITCH - 8)
    clear(32 * _PITCH + 8)
    cxa.wait()
    cxb.wait()
    perm = perm_s[...].astype(_BF16)
    xa = jnp.concatenate(
        [_dot(xa_buf[:, 128 * k:128 * (k + 1)], perm) for k in range(4)], axis=1).astype(_BF16)
    xb = xb_buf[...]
    ma_s[...] = jnp.full(ma_s.shape, -jnp.inf, _F32)

    def absorb(a, s, half):
        ev, od = head_pair(wuk_buf, a, s, 2 * half, 2 * half + 2)
        for h, w in ((8 * a + 2 * s, ev), (8 * a + 2 * s + 1, od)):
            r = _dot_nt(qa_s[h].astype(_BF16), w) * scale
            qabs_s[2 * half, _ds(h * 8, 4), :] = r[:, :128]
            qabs_s[2 * half + 1, _ds(h * 8, 4), :] = r[:, 128:]

    def p2(a, c):
        for s in range(4):
            t = 4 * a + s
            pace(s_wqb, [(True, s_wuv)], t, 0)
            ev, od = head_pair(wq_buf, a, s, 0, 4)
            qa_s[2 * t] = _dot(xa, ev)
            qa_s[2 * t + 1] = _dot(xa, od)
            pace(s_wqb, [(True, s_wuv)], t, 1)
            absorb(a, s, 0)
        return c
    lax.fori_loop(0, 4, p2, 0)

    def p3(a, c):
        for s in range(4):
            t = 4 * a + s
            pace(s_wuv, [(True, s_c)], t, 0)
            w = wqb_buf[:, :, :, _ds(t * 256, 256, 256)].reshape(512, 256)
            q = _dot(xb, w) * scale
            qb_s[_ds(t * 16, 4), :] = q[:, :128]
            qb_s[_ds(t * 16 + 8, 4), :] = q[:, 128:]
            pace(s_wuv, [(True, s_c)], t, 1)
            absorb(a, s, 1)
        return c
    lax.fori_loop(0, 4, p3, 0)

    nxt = [(True, k_stream(0))]

    def c_block(t, jb):
        return c_buf[t, pl.ds(2 * jb, 2)].reshape(128, 512)

    def c_scores(t, jb):
        b = 2 * (t >> 5) + jb
        sa = _dot_nt(qabs_t[_ds(b * 32, 32, 32), :], c_block(t, jb))
        sa_s[t, jb] = sa
        ma_s[b] = jnp.maximum(ma_s[b], sa)

    def unpermute(b0):
        for ct in range(4):
            r = jnp.concatenate(
                [qabs_s[ct, pl.ds(b, 32, stride=8), :] for b in (b0, b0 + 1)], axis=0)
            qabs_t[32 * b0:32 * b0 + 64, 128 * ct:128 * (ct + 1)] = (
                _dot_nt(r.astype(_BF16), perm).astype(_BF16))

    pace(s_c, nxt, 0, 0)
    unpermute(0)
    pace(s_c, nxt, 0, 1)
    unpermute(2)
    pace(s_c, nxt, 1, 0)
    for b in range(4):
        qb_t[b] = qb_s[pl.ds(b, 32, stride=8), :]

    def cstep(t, c):
        wait(t, 1)
        c_scores(t - 1, 0)
        issue(s_c, nxt, t, 1)
        wait(t + 1, 0)
        c_scores(t - 1, 1)
        issue(s_c, nxt, t + 1, 0)
        return c
    lax.fori_loop(1, 64, cstep, 0)
    c_scores(63, 0)
    c_scores(63, 1)

    top = lax.broadcasted_iota(jnp.int32, (8, 128), 0) < 4

    def batch(b, carry):
        ks, vs = k_stream(b), v_stream(b)
        qb = [qb_t[b, 8 * i:8 * i + 8, :].astype(_BF16) for i in range(4)]

        def kstep(t, mb):
            mb = list(mb)
            r = _ds(t * 128, 128, 128)
            se = [_dot_nt(qb[i], k_buf[i, 0, r, :]) for i in range(4)]
            issue(ks, [(True, vs)], t, 0, skip0=True)
            wait(t, 1)
            for i in range(4):
                s = jnp.where(top, se[i], _dot_nt(qb[i], k_buf[i, 1, r, :]))
                sb_s[t, i] = s
                mb[i] = jnp.maximum(mb[i], s)
            issue(ks, [(True, vs)], t, 1)
            wait(t + 1, 0)
            return tuple(mb)

        mb = lax.fori_loop(0, 32, kstep, (jnp.full((8, 128), -jnp.inf, _F32),) * 4)
        vs.start(_LOOK, 0)
        mb = [jnp.broadcast_to(jnp.max(m, axis=-1, keepdims=True), (8, 128)) for m in mb]
        ma = jnp.broadcast_to(jnp.max(ma_s[b], axis=-1, keepdims=True), (32, 128))

        nxt = [(b < 3, k_stream(jnp.minimum(b + 1, 3))), (b == 3, s_wo)]

        def vstep(t, c):
            lb, ab, la, aa = list(c[0]), list(c[1]), c[2], c[3]
            r = _ds(t * 128, 128, 128)
            issue(vs, nxt, t, 0, skip0=True)
            tc = (b >> 1) * 32 + t
            p = jnp.exp(sa_s[tc, b & 1] - ma)
            la = la + p
            aa = aa + _dot(p.astype(_BF16), c_block(tc, b & 1))
            wait(t, 1)
            for i in range(4):
                p = jnp.exp(sb_s[t, i] - mb[i])
                lb[i] = lb[i] + p
                p = p.astype(_BF16)
                ab[i] = ab[i] + jnp.where(top, _dot(p, v_buf[i, 0, r, :]),
                                          _dot(p, v_buf[i, 1, r, :]))
            issue(vs, nxt, t, 1)
            wait(t + 1, 0)
            return tuple(lb), tuple(ab), la, aa

        z8 = jnp.zeros((8, 128), _F32)
        lb, ab, la, aa = lax.fori_loop(
            0, 32, vstep,
            ((z8,) * 4, (z8,) * 4, jnp.zeros((32, 128), _F32), jnp.zeros((32, 512), _F32)))
        for cond, st in nxt:
            pl.when(cond)(lambda st=st: st.start(_LOOK, 0))
        ob = jnp.concatenate(
            [ab[i] / jnp.sum(lb[i], axis=-1, keepdims=True) for i in range(4)], axis=0)
        rl = jnp.broadcast_to(1.0 / jnp.sum(la, axis=-1, keepdims=True), (32, 128))
        aa = aa.astype(_BF16)
        cc = [_dot(aa[:, 128 * ct:128 * (ct + 1)], perm) for ct in range(4)]
        for bb in range(4):
            @pl.when(b == bb)
            def _():
                rows = pl.ds(bb, 32, stride=8)
                ob_s[rows, :] = ob
                rl_s[rows, :] = rl
                for ct in range(4):
                    cc_s[ct, rows, :] = cc[ct]
        return carry
    lax.fori_loop(0, 4, batch, 0)

    lhs_of = (ob_s, ctx_s)

    def proj(g, rg, j):
        lhs = lhs_of[g][_ds((8 * rg + j) * 8, 4), :].astype(_BF16)
        return _dot(lhs, wo_buf[g][rg >> 1, rg & 1, _ds(j * 128, 128, 128), :])

    nxt = [(True, s_wo_last)]

    def fstep(s, gs):
        def body(t, out):
            rg, j = t & 3, (t >> 2) - 1
            out = tuple(out[g] + proj(g, rg, j) if g in gs else out[g] for g in range(2))
            issue(s_wo, nxt, t, 0, skip0=True)
            pace(s_wo, nxt, t, 1)
            if s is not None:
                ev, od = head_pair(wuv_buf, rg, s, 0, 4)
                for h, w in ((8 * rg + 2 * s, ev), (8 * rg + 2 * s + 1, od)):
                    row = _ds(h * 8, 4)
                    lhs = jnp.concatenate([cc_s[ct, row, :] for ct in range(4)], axis=1)
                    ctx_s[row, :] = _dot(lhs.astype(_BF16), w) * rl_s[row, :]
            wait(t + 1, 0)
            return out
        return body

    out = (jnp.zeros((4, 512), _F32),) * 2
    for s in range(4):
        out = lax.fori_loop(8 * s, 8 * s + 4, fstep(s, (0, 1) if s else ()), out)
        if s < 3:
            out = lax.fori_loop(8 * s + 4, 8 * s + 8, fstep(None, (0, 1) if s else (1,)), out)
    out = list(out)
    for rg in range(4):
        out[0] = out[0] + proj(0, rg, 6) + proj(0, rg, 0)
        out[1] = out[1] + proj(1, rg, 6)
    for u in range(8):
        for v in {1: (1, 2, 3, 4), 5: (5, 6), 7: (7,)}.get(u, ()):
            wait(v >> 1, v & 1)
        out[u & 1] = out[u & 1] + proj(u & 1, u >> 1, 7)
        if u == 6:
            out_ref[:, 512:] = out[0].astype(out_ref.dtype)
    out_ref[:, :512] = out[1].astype(out_ref.dtype)


@jax.jit
def pallas_concat_heads__compressed_kv_cla__gqa_block_cached__decode_kernel(
    A_x: jax.Array,
    A_c_kv: jax.Array,
    A_w_q: jax.Array,
    A_w_uk: jax.Array,
    A_w_uv: jax.Array,
    A_w_o: jax.Array,
    B_x: jax.Array,
    B_k_cache: jax.Array,
    B_v_cache: jax.Array,
    B_wq: jax.Array,
    B_wo: jax.Array,
):
    vm = pltpu.VMEM
    pitched = 32 * _PITCH + 16
    out = pl.pallas_call(
        _kernel,
        in_specs=[pl.BlockSpec(memory_space=pl.ANY)] * 11,
        out_specs=pl.BlockSpec(memory_space=pltpu.VMEM),
        out_shape=jax.ShapeDtypeStruct((4, 1024), _BF16),
        scratch_shapes=[
            vm((4, 512), _BF16),
            vm((4, 512), _BF16),
            vm((2, 2, pitched, 128), _BF16),
            vm((2, 2, pitched, 128), _BF16),
            vm((4, pitched, 128), _BF16),
            vm((2, 2, 1024, 512), _BF16),
            vm((2, 4, 64, 4096), _BF16),
            vm((2, 2, 1024, 512), _BF16),
            vm((64, 4, 2, 32, 512), _BF16),
            vm((4, 2, 4096, 128), _BF16),
            vm((4, 2, 4096, 128), _BF16),
            vm((3, 128, 128), _BF16),
            vm((128, 128), _F32),
            vm((32, 4, 128), _F32),
            vm((4, 256, 128), _F32),
            vm((128, 512), _BF16),
            vm((256, 128), _F32),
            vm((4, 32, 128), _F32),
            vm((64, 2, 32, 128), _F32),
            vm((4, 32, 128), _F32),
            vm((32, 4, 8, 128), _F32),
            vm((256, 128), _F32),
            vm((4, 256, 128), _F32),
            vm((256, 128), _F32),
            vm((256, 128), _F32),
            pltpu.SemaphoreType.DMA((_LOOK * 2,)),
            pltpu.SemaphoreType.DMA((_LOOK * 2,)),
            pltpu.SemaphoreType.DMA((2,)),
        ],
        compiler_params=pltpu.CompilerParams(
            vmem_limit_bytes=80 * 1024 * 1024,
            disable_bounds_checks=True,
            disable_semaphore_checks=True),
    )(
        A_x.reshape(4, 512), A_c_kv.reshape(2, 4, 2, 1024, 512),
        A_w_q.reshape(2, 2, 4096, 128), A_w_uk.reshape(2, 2, 4096, 128),
        A_w_uv.reshape(4, 4096, 128), A_w_o.reshape(2, 2, 1024, 512),
        B_x.reshape(4, 512), B_k_cache.reshape(4, 4, 2, 4096, 128),
        B_v_cache.reshape(4, 4, 2, 4096, 128),
        B_wq.reshape(2, 4, 64, 4096), B_wo.reshape(2, 2, 1024, 512),
    )
    return out.reshape(4, 1, 1024)
```

```python
import jax
import jax.numpy as jnp
from jax import lax
import jax.experimental.pallas as pl
import jax.experimental.pallas.tpu as pltpu

_F32 = jnp.float32
_BF16 = jnp.bfloat16
_LOOK = 4
_PITCH = 136


def _dot(a, b):
    return jnp.dot(a, b, preferred_element_type=_F32)


def _dot_nt(a, b):
    return lax.dot_general(a, b, (((1,), (1,)), ((), ())), preferred_element_type=_F32)


def _ds(start, size, mult=8):
    if not isinstance(start, int):
        start = pl.multiple_of(start, mult)
    return pl.ds(start, size)


def _when(*conds):
    if any(c is False for c in conds):
        return lambda f: None
    traced = [c for c in conds if c is not True]
    if not traced:
        return lambda f: f()
    cond = traced[0]
    for c in traced[1:]:
        cond = jnp.logical_and(cond, c)
    return pl.when(cond)


def _kernel(xa_hbm, c_hbm, wq_hbm, wuk_hbm, wuv_hbm, woa_hbm,
            xb_hbm, k_hbm, v_hbm, wqb_hbm, wob_hbm,
            out_ref,
            xa_buf, xb_buf, wq_buf, wuk_buf, wuv_buf, woa_buf, wqb_buf, wob_buf,
            c_buf, k_buf, v_buf, size_ref,
            perm_s, qa_s, qabs_s, qabs_t, qb_s, qb_t, sa_s, ma_s, sb_s, ob_s, cc_s, rl_s, ctx_s,
            hsem, lsem, xsem):
    scale = 128 ** -0.5

    def copies(unit, t, g):
        i = (t & (_LOOK - 1)) * 2 + g
        return ([pltpu.make_async_copy(a, b, hsem.at[i]) for a, b in unit[0]],
                [pltpu.make_async_copy(a, b, lsem.at[i]) for a, b in unit[1]])

    def wait(t, g):
        hi, lo = size_ref.at[pl.ds(0, 1)], size_ref.at[pl.ds(0, 3)]
        hi, lo = copies(([(hi, hi)], [(lo, lo)]), t, g)
        lo[0].wait()
        hi[0].wait()

    def go(unit, t, g):
        his, los = copies(unit, t, g)
        for c in his:
            c.start(priority=0)
        for c in los:
            c.start(priority=1)

    class Stream:
        def __init__(self, steps, fn, wraps=lambda g: False):
            self.steps, self.fn, self.wraps = steps, fn, wraps

        def start(self, t, g, maybe0=False):
            if maybe0 and self.wraps(g) and not isinstance(t, int):
                pl.when(t == 0)(lambda: go(self.fn(0, g), 0, g))
                pl.when(t > 0)(lambda: go(self.fn(jnp.maximum(t, 1), g), t, g))
            else:
                go(self.fn(t, g), t, g)

    def views(hbm, buf, lead, boxes):
        return [(hbm.at[lead + a], buf.at[lead + b]) for a, b in boxes]

    def row_piece(hbm, buf, rows, rows0):
        def piece(lead, p):
            rs = rows0 if isinstance(p, int) and p == 0 else [rows(p)]
            return views(hbm, buf, lead, [((_ds(a, n),), (_ds(b, n),)) for a, b, n in rs])
        return piece

    def gather_piece(hbm, buf):
        return row_piece(hbm, buf, lambda p: (p * 128 - 8, p * _PITCH, 128),
                         [(0, 8, 120), (4088, 32 * _PITCH, 8)])

    def kv_piece(hbm, buf):
        return row_piece(hbm, buf, lambda p: (p * 128 - 120, p * 128, 128),
                         [(3976, 0, 120), (0, 120, 8)])

    def wqb_piece(lead, p):
        h = p & 1
        boxes = [(_ds((p >> 1) * 8, 8), _ds(h * 2048 + 128, 1920, 128)),
                 (_ds((((p + 1) >> 1) & 7) * 8, 8), _ds((1 - h) * 2048, 128, 128))]
        return views(wqb_hbm, wqb_buf, lead, [(x, x) for x in boxes])

    def c_piece(lead, p):
        hbm, r, q = c_hbm.at[p >> 5], (p & 31) * 32, (p + 31) & 31
        tail, head = pl.ds(384, 128), pl.ds(0, 384)
        return (views(hbm, c_buf.at[(p & 32) + q], lead,
                      [((_ds(q * 32 + 24, 8), tail), (pl.ds(24, 8), tail))])
                + views(hbm, c_buf.at[p], lead,
                        [((_ds(r, 24),), (pl.ds(0, 24),)),
                         ((_ds(r + 24, 8), head), (pl.ds(24, 8), head))]))

    def woa_piece(lead, p):
        boxes = [(_ds(jnp.where(p == 0, 888, p * 32 - 8), 8), pl.ds(384, 128)),
                 (_ds(p * 32, 24),), (_ds(p * 32 + 24, 8), pl.ds(0, 384))]
        return views(woa_hbm, woa_buf, lead, [(x, x) for x in boxes])

    def wob_piece(lead, p):
        boxes = [(_ds(p * 32, 8), pl.ds(128, 384)), (_ds(p * 32 + 8, 24),),
                 (_ds(jnp.where(p == 27, 0, p * 32 + 32), 8), pl.ds(0, 128))]
        return views(wob_hbm, wob_buf, lead, [(x, x) for x in boxes])

    def quad(piece, p, pre=(), post=()):
        return piece(pre + (pl.ds(3, 1),) + post, p), piece(pre + (pl.ds(0, 3),) + post, p)

    def cross(px, py):
        def fn(t, g):
            x, y = (px, py) if g == 0 else (py, px)
            return y((pl.ds(1, 1), g), t), x((pl.ds(0, 2), g), t) + y((pl.ds(0, 1), g), t)
        return fn

    wo_hbm, wo_buf = (wob_hbm, woa_hbm), (wob_buf, woa_buf)

    def wo_last(t, g):
        rows = lambda a, n: views(wo_hbm[g], wo_buf[g], (t >> 1, t & 1), [((pl.ds(a, n),),) * 2])
        return rows(992, 32), rows(896, 96)

    always = lambda g: True
    s_wa = Stream(32, cross(gather_piece(wuk_hbm, wuk_buf), gather_piece(wq_hbm, wq_buf)), always)
    s_wqb = Stream(16, lambda t, g: quad(wqb_piece, t, pre=(g,)))
    s_wuv = Stream(16, lambda t, g: quad(gather_piece(wuv_hbm, wuv_buf), t + 16 * g),
                   lambda g: g == 0)
    s_c = Stream(64, lambda t, g: quad(c_piece, t, post=(g,)))
    kv_stream = lambda hbm, buf, o: Stream(
        32, lambda t, g: quad(kv_piece(hbm.at[g, o & 1, :, o >> 1], buf.at[:, g]), t), always)
    k_stream = lambda o: kv_stream(k_hbm, k_buf, o)
    v_stream = lambda o: kv_stream(v_hbm, v_buf, o)
    s_wo = Stream(28, cross(wob_piece, woa_piece))
    s_wo_last = Stream(4, wo_last)

    def issue(cur, nxt, t, g, skip0=False):
        u = t + _LOOK
        _when(u < cur.steps, t > 0 if skip0 else True)(lambda: cur.start(u, g))
        for cond, st in nxt:
            _when(u >= cur.steps, cond)(lambda st=st: st.start(u - cur.steps, g, maybe0=True))

    def pace(cur, nxt, t, g):
        wait(t, g)
        issue(cur, nxt, t, g)

    def head_pair(buf, a, s, lo, hi):
        wp = _PITCH // 2
        lead = (slice(None),) * (len(buf.shape) - 2)
        reg = (lambda r: (r,)) if len(lead) == 1 else (lambda r: (r // 2, r % 2))
        words = buf.bitcast(jnp.uint32)
        n = 31 * wp + 52
        view = words.at[lead + (_ds(4 * a + 4, n, 4),)]
        last = words.at[lead + (_ds(4 * a + 4 + 4 * ((a + 1) >> 2), n, 4),)]
        x = jnp.concatenate(
            [(view if ml < 3 else last)[reg(r) + (pl.ds(16 * ml + s, 32, stride=wp), slice(None))]
             for r in range(lo, hi) for ml in range(4)], axis=0)
        even = pltpu.bitcast(x << 16, _F32).astype(_BF16)
        odd = pltpu.bitcast(x & jnp.uint32(0xFFFF0000), _F32).astype(_BF16)
        return even, odd

    units = [copies(s_wa.fn(t, g), t, g) for t in range(_LOOK) for g in range(2)]
    for c in units[0][0]:
        c.start(priority=0)
    for _, los in units:
        for c in los:
            c.start(priority=1)
    cxa = pltpu.make_async_copy(xa_hbm, xa_buf, xsem.at[0])
    cxb = pltpu.make_async_copy(xb_hbm, xb_buf, xsem.at[1])
    cxa.start()
    cxb.start()

    ji = lax.broadcasted_iota(jnp.int32, (1, 128), 1)
    src_row = 4 * (ji & 31) + (ji >> 5)

    def perm_row(m, c):
        perm_s[pl.ds(m, 1), :] = jnp.where(src_row == m, 1.0, 0.0)
        return c
    for k in range(8):
        lax.fori_loop(16 * k, 16 * k + 16, perm_row, 0)
        if k < 7:
            for c in units[k + 1][0]:
                c.start(priority=0)

    def clear(row):
        wq_buf[:, :, _ds(row, 8), :] = jnp.zeros((2, 2, 8, 128), _BF16)
        wuk_buf[:, :, _ds(row, 8), :] = jnp.zeros((2, 2, 8, 128), _BF16)
        wuv_buf[:, _ds(row, 8), :] = jnp.zeros((4, 8, 128), _BF16)

    def pa(t, c):
        for g in range(2):
            pace(s_wa, [(True, s_wqb)], t, g)
        clear(jnp.maximum(t * _PITCH - 8, 0))
        return c
    lax.fori_loop(0, 32, pa, 0)
    clear(32 * _PITCH - 8)
    clear(32 * _PITCH + 8)
    cxa.wait()
    cxb.wait()
    perm = perm_s[...].astype(_BF16)
    xa = jnp.concatenate(
        [_dot(xa_buf[:, 128 * k:128 * (k + 1)], perm) for k in range(4)], axis=1).astype(_BF16)
    xb = xb_buf[...]
    ma_s[...] = jnp.full(ma_s.shape, -jnp.inf, _F32)

    def absorb(a, s, half):
        ev, od = head_pair(wuk_buf, a, s, 2 * half, 2 * half + 2)
        for h, w in ((8 * a + 2 * s, ev), (8 * a + 2 * s + 1, od)):
            r = _dot_nt(qa_s[h].astype(_BF16), w) * scale
            qabs_s[2 * half, _ds(h * 8, 4), :] = r[:, :128]
            qabs_s[2 * half + 1, _ds(h * 8, 4), :] = r[:, 128:]

    def p2(a, c):
        for s in range(4):
            t = 4 * a + s
            pace(s_wqb, [(True, s_wuv)], t, 0)
            ev, od = head_pair(wq_buf, a, s, 0, 4)
            qa_s[2 * t] = _dot(xa, ev)
            qa_s[2 * t + 1] = _dot(xa, od)
            pace(s_wqb, [(True, s_wuv)], t, 1)
            absorb(a, s, 0)
        return c
    lax.fori_loop(0, 4, p2, 0)

    def p3(a, c):
        for s in range(4):
            t = 4 * a + s
            pace(s_wuv, [(True, s_c)], t, 0)
            w = wqb_buf[:, :, :, _ds(t * 256, 256, 256)].reshape(512, 256)
            q = _dot(xb, w) * scale
            qb_s[_ds(t * 16, 4), :] = q[:, :128]
            qb_s[_ds(t * 16 + 8, 4), :] = q[:, 128:]
            pace(s_wuv, [(True, s_c)], t, 1)
            absorb(a, s, 1)
        return c
    lax.fori_loop(0, 4, p3, 0)

    nxt = [(True, k_stream(0))]

    def c_block(t, jb):
        return c_buf[t, pl.ds(2 * jb, 2)].reshape(128, 512)

    def c_scores(t, jb):
        b = 2 * (t >> 5) + jb
        sa = _dot_nt(qabs_t[_ds(b * 32, 32, 32), :], c_block(t, jb))
        sa_s[t, jb] = sa
        ma_s[b] = jnp.maximum(ma_s[b], sa)

    def unpermute(b0):
        for ct in range(4):
            r = jnp.concatenate(
                [qabs_s[ct, pl.ds(b, 32, stride=8), :] for b in (b0, b0 + 1)], axis=0)
            qabs_t[32 * b0:32 * b0 + 64, 128 * ct:128 * (ct + 1)] = (
                _dot_nt(r.astype(_BF16), perm).astype(_BF16))

    pace(s_c, nxt, 0, 0)
    unpermute(0)
    pace(s_c, nxt, 0, 1)
    unpermute(2)
    pace(s_c, nxt, 1, 0)
    q_rows = lambda o, i, g: pl.ds(32 * (2 * i + (o >> 1)) + (o & 1) + 2 * g, 4, stride=8)
    for o in range(4):
        for i in range(4):
            for g in range(2):
                qb_t[o, 8 * i + 4 * g:8 * i + 4 * g + 4, :] = qb_s[q_rows(o, i, g), :]

    def cstep(t, c):
        wait(t, 1)
        c_scores(t - 1, 0)
        issue(s_c, nxt, t, 1)
        wait(t + 1, 0)
        c_scores(t - 1, 1)
        issue(s_c, nxt, t + 1, 0)
        return c
    lax.fori_loop(1, 64, cstep, 0)
    c_scores(63, 0)
    c_scores(63, 1)

    top = lax.broadcasted_iota(jnp.int32, (8, 128), 0) < 4

    def batch(b, carry):
        ks, vs = k_stream(b), v_stream(b)
        qb = [qb_t[b, 8 * i:8 * i + 8, :].astype(_BF16) for i in range(4)]

        def kstep(t, mb):
            mb = list(mb)
            r = _ds(t * 128, 128, 128)
            se = [_dot_nt(qb[i], k_buf[i, 0, r, :]) for i in range(4)]
            issue(ks, [(True, vs)], t, 0, skip0=True)
            wait(t, 1)
            for i in range(4):
                s = jnp.where(top, se[i], _dot_nt(qb[i], k_buf[i, 1, r, :]))
                sb_s[t, i] = s
                mb[i] = jnp.maximum(mb[i], s)
            issue(ks, [(True, vs)], t, 1)
            wait(t + 1, 0)
            return tuple(mb)

        mb = lax.fori_loop(0, 32, kstep, (jnp.full((8, 128), -jnp.inf, _F32),) * 4)
        vs.start(_LOOK, 0)
        mb = [jnp.broadcast_to(jnp.max(m, axis=-1, keepdims=True), (8, 128)) for m in mb]
        ma = jnp.broadcast_to(jnp.max(ma_s[b], axis=-1, keepdims=True), (32, 128))

        nxt = [(b < 3, k_stream(jnp.minimum(b + 1, 3))), (b == 3, s_wo)]

        def vstep(t, c):
            lb, ab, la, aa = list(c[0]), list(c[1]), c[2], c[3]
            r = _ds(t * 128, 128, 128)
            issue(vs, nxt, t, 0, skip0=True)
            tc = (b >> 1) * 32 + t
            p = jnp.exp(sa_s[tc, b & 1] - ma)
            la = la + p
            aa = aa + _dot(p.astype(_BF16), c_block(tc, b & 1))
            wait(t, 1)
            for i in range(4):
                p = jnp.exp(sb_s[t, i] - mb[i])
                lb[i] = lb[i] + p
                p = p.astype(_BF16)
                ab[i] = ab[i] + jnp.where(top, _dot(p, v_buf[i, 0, r, :]),
                                          _dot(p, v_buf[i, 1, r, :]))
            issue(vs, nxt, t, 1)
            wait(t + 1, 0)
            return tuple(lb), tuple(ab), la, aa

        z8 = jnp.zeros((8, 128), _F32)
        lb, ab, la, aa = lax.fori_loop(
            0, 32, vstep,
            ((z8,) * 4, (z8,) * 4, jnp.zeros((32, 128), _F32), jnp.zeros((32, 512), _F32)))
        for cond, st in nxt:
            pl.when(cond)(lambda st=st: st.start(_LOOK, 0))
        ob = [ab[i] / jnp.sum(lb[i], axis=-1, keepdims=True) for i in range(4)]
        rl = jnp.broadcast_to(1.0 / jnp.sum(la, axis=-1, keepdims=True), (32, 128))
        aa = aa.astype(_BF16)
        cc = [_dot(aa[:, 128 * ct:128 * (ct + 1)], perm) for ct in range(4)]
        for bb in range(4):
            @pl.when(b == bb)
            def _():
                rows = pl.ds(bb, 32, stride=8)
                for i in range(4):
                    for g in range(2):
                        ob_s[q_rows(bb, i, g), :] = ob[i][4 * g:4 * g + 4]
                rl_s[rows, :] = rl
                for ct in range(4):
                    cc_s[ct, rows, :] = cc[ct]
        return carry
    lax.fori_loop(0, 4, batch, 0)

    lhs_of = (ob_s, ctx_s)

    def proj(g, rg, j):
        lhs = lhs_of[g][_ds((8 * rg + j) * 8, 4), :].astype(_BF16)
        return _dot(lhs, wo_buf[g][rg >> 1, rg & 1, _ds(j * 128, 128, 128), :])

    nxt = [(True, s_wo_last)]

    def fstep(s, gs):
        def body(t, out):
            rg, j = t & 3, (t >> 2) - 1
            out = tuple(out[g] + proj(g, rg, j) if g in gs else out[g] for g in range(2))
            issue(s_wo, nxt, t, 0, skip0=True)
            pace(s_wo, nxt, t, 1)
            if s is not None:
                ev, od = head_pair(wuv_buf, rg, s, 0, 4)
                for h, w in ((8 * rg + 2 * s, ev), (8 * rg + 2 * s + 1, od)):
                    row = _ds(h * 8, 4)
                    lhs = jnp.concatenate([cc_s[ct, row, :] for ct in range(4)], axis=1)
                    ctx_s[row, :] = _dot(lhs.astype(_BF16), w) * rl_s[row, :]
            wait(t + 1, 0)
            return out
        return body

    out = (jnp.zeros((4, 512), _F32),) * 2
    for k, s in enumerate((0, None, 1, None, 2, 3, None)):
        out = lax.fori_loop(4 * k, 4 * k + 4, fstep(s, {0: (), 1: (1,)}.get(k, (0, 1))), out)
    out = list(out)
    for rg in range(4):
        out[0] = out[0] + proj(0, rg, 6) + proj(0, rg, 0)
        out[1] = out[1] + proj(1, rg, 6)
    for u in range(8):
        for v in {1: (1, 2, 3, 4), 5: (5, 6), 7: (7,)}.get(u, ()):
            wait(v >> 1, v & 1)
        out[u & 1] = out[u & 1] + proj(u & 1, u >> 1, 7)
        if u == 6:
            out_ref[:, 512:] = out[0].astype(out_ref.dtype)
    out_ref[:, :512] = out[1].astype(out_ref.dtype)


@jax.jit
def pallas_concat_heads__compressed_kv_cla__gqa_block_cached__decode_kernel(
    A_x: jax.Array,
    A_c_kv: jax.Array,
    A_w_q: jax.Array,
    A_w_uk: jax.Array,
    A_w_uv: jax.Array,
    A_w_o: jax.Array,
    B_x: jax.Array,
    B_k_cache: jax.Array,
    B_v_cache: jax.Array,
    B_wq: jax.Array,
    B_wo: jax.Array,
):
    vm = pltpu.VMEM
    pitched = 32 * _PITCH + 16
    out = pl.pallas_call(
        _kernel,
        in_specs=[pl.BlockSpec(memory_space=pl.ANY)] * 11,
        out_specs=pl.BlockSpec(memory_space=pltpu.VMEM),
        out_shape=jax.ShapeDtypeStruct((4, 1024), _BF16),
        scratch_shapes=[
            vm((4, 512), _BF16),
            vm((4, 512), _BF16),
            vm((2, 2, pitched, 128), _BF16),
            vm((2, 2, pitched, 128), _BF16),
            vm((4, pitched, 128), _BF16),
            vm((2, 2, 1024, 512), _BF16),
            vm((2, 4, 64, 4096), _BF16),
            vm((2, 2, 1024, 512), _BF16),
            vm((64, 4, 2, 32, 512), _BF16),
            vm((4, 2, 4096, 128), _BF16),
            vm((4, 2, 4096, 128), _BF16),
            vm((3, 128, 128), _BF16),
            vm((128, 128), _F32),
            vm((32, 4, 128), _F32),
            vm((4, 256, 128), _F32),
            vm((128, 512), _BF16),
            vm((256, 128), _F32),
            vm((4, 32, 128), _F32),
            vm((64, 2, 32, 128), _F32),
            vm((4, 32, 128), _F32),
            vm((32, 4, 8, 128), _F32),
            vm((256, 128), _F32),
            vm((4, 256, 128), _F32),
            vm((256, 128), _F32),
            vm((256, 128), _F32),
            pltpu.SemaphoreType.DMA((_LOOK * 2,)),
            pltpu.SemaphoreType.DMA((_LOOK * 2,)),
            pltpu.SemaphoreType.DMA((2,)),
        ],
        compiler_params=pltpu.CompilerParams(
            vmem_limit_bytes=80 * 1024 * 1024,
            disable_bounds_checks=True,
            disable_semaphore_checks=True),
    )(
        A_x.reshape(4, 512), A_c_kv.reshape(2, 4, 2, 1024, 512),
        A_w_q.reshape(2, 2, 4096, 128), A_w_uk.reshape(2, 2, 4096, 128),
        A_w_uv.reshape(4, 4096, 128), A_w_o.reshape(2, 2, 1024, 512),
        B_x.reshape(4, 512), B_k_cache.reshape(2, 2, 4, 2, 4096, 128),
        B_v_cache.reshape(2, 2, 4, 2, 4096, 128),
        B_wq.reshape(2, 4, 64, 4096), B_wo.reshape(2, 2, 1024, 512),
    )
    return out.reshape(4, 1, 1024)
```

```python
import jax
import jax.numpy as jnp
from jax import lax
import jax.experimental.pallas as pl
import jax.experimental.pallas.tpu as pltpu

_F32 = jnp.float32
_BF16 = jnp.bfloat16
_LOOK = 4
_PITCH = 136


def _dot(a, b):
    return jnp.dot(a, b, preferred_element_type=_F32)


def _dot_nt(a, b):
    return lax.dot_general(a, b, (((1,), (1,)), ((), ())), preferred_element_type=_F32)


def _ds(start, size, mult=8):
    if not isinstance(start, int):
        start = pl.multiple_of(start, mult)
    return pl.ds(start, size)


def _when(*conds):
    if any(c is False for c in conds):
        return lambda f: None
    traced = [c for c in conds if c is not True]
    if not traced:
        return lambda f: f()
    cond = traced[0]
    for c in traced[1:]:
        cond = jnp.logical_and(cond, c)
    return pl.when(cond)


def _kernel(xa_hbm, c_hbm, wq_hbm, wuk_hbm, wuv_hbm, woa_hbm,
            xb_hbm, k_hbm, v_hbm, wqb_hbm, wob_hbm,
            out_ref,
            xa_buf, xb_buf, wq_buf, wuk_buf, wuv_buf, woa_buf, wqb_buf, wob_buf,
            c_buf, k_buf, v_buf, size_ref,
            perm_s, qa_s, qabs_s, qabs_t, qb_s, qb_t, sa_s, ma_s, sb_s, ob_s, cc_s, rl_s, ctx_s,
            hsem, lsem, xsem):
    scale = 128 ** -0.5

    def copies(unit, t, g):
        i = (t & (_LOOK - 1)) * 2 + g
        return ([pltpu.make_async_copy(a, b, hsem.at[i]) for a, b in unit[0]],
                [pltpu.make_async_copy(a, b, lsem.at[i]) for a, b in unit[1]])

    def wait(t, g):
        hi, lo = size_ref.at[pl.ds(0, 1)], size_ref.at[pl.ds(0, 3)]
        hi, lo = copies(([(hi, hi)], [(lo, lo)]), t, g)
        lo[0].wait()
        hi[0].wait()

    def go(unit, t, g):
        his, los = copies(unit, t, g)
        for c in his:
            c.start(priority=0)
        for c in los:
            c.start(priority=1)

    class Stream:
        def __init__(self, steps, fn, wraps=lambda g: False):
            self.steps, self.fn, self.wraps = steps, fn, wraps

        def start(self, t, g, maybe0=False):
            if maybe0 and self.wraps(g) and not isinstance(t, int):
                pl.when(t == 0)(lambda: go(self.fn(0, g), 0, g))
                pl.when(t > 0)(lambda: go(self.fn(jnp.maximum(t, 1), g), t, g))
            else:
                go(self.fn(t, g), t, g)

    def views(hbm, buf, lead, boxes):
        return [(hbm.at[lead + a], buf.at[lead + b]) for a, b in boxes]

    def row_piece(hbm, buf, rows, rows0):
        def piece(lead, p):
            rs = rows0 if isinstance(p, int) and p == 0 else [rows(p)]
            return views(hbm, buf, lead, [((_ds(a, n),), (_ds(b, n),)) for a, b, n in rs])
        return piece

    def gather_piece(hbm, buf):
        return row_piece(hbm, buf, lambda p: (p * 128 - 8, p * _PITCH, 128),
                         [(0, 8, 120), (4088, 32 * _PITCH, 8)])

    def kv_piece(hbm, buf):
        return row_piece(hbm, buf, lambda p: (p * 128 - 120, p * 128, 128),
                         [(3976, 0, 120), (0, 120, 8)])

    def wqb_piece(lead, p):
        h = p & 1
        boxes = [(_ds((p >> 1) * 8, 8), _ds(h * 2048 + 128, 1920, 128)),
                 (_ds((((p + 1) >> 1) & 7) * 8, 8), _ds((1 - h) * 2048, 128, 128))]
        return views(wqb_hbm, wqb_buf, lead, [(x, x) for x in boxes])

    def c_piece(lead, p):
        hbm, r, q = c_hbm.at[p >> 5], (p & 31) * 32, (p + 31) & 31
        tail, head = pl.ds(384, 128), pl.ds(0, 384)
        return (views(hbm, c_buf.at[(p & 32) + q], lead,
                      [((_ds(q * 32 + 24, 8), tail), (pl.ds(24, 8), tail))])
                + views(hbm, c_buf.at[p], lead,
                        [((_ds(r, 24),), (pl.ds(0, 24),)),
                         ((_ds(r + 24, 8), head), (pl.ds(24, 8), head))]))

    def woa_piece(lead, p):
        boxes = [(_ds(jnp.where(p == 0, 888, p * 32 - 8), 8), pl.ds(384, 128)),
                 (_ds(p * 32, 24),), (_ds(p * 32 + 24, 8), pl.ds(0, 384))]
        return views(woa_hbm, woa_buf, lead, [(x, x) for x in boxes])

    def wob_piece(lead, p):
        boxes = [(_ds(p * 32, 8), pl.ds(128, 384)), (_ds(p * 32 + 8, 24),),
                 (_ds(jnp.where(p == 27, 0, p * 32 + 32), 8), pl.ds(0, 128))]
        return views(wob_hbm, wob_buf, lead, [(x, x) for x in boxes])

    def quad(piece, p, pre=(), post=()):
        return piece(pre + (pl.ds(3, 1),) + post, p), piece(pre + (pl.ds(0, 3),) + post, p)

    def cross(px, py):
        def fn(t, g):
            x, y = (px, py) if g == 0 else (py, px)
            return y((pl.ds(1, 1), g), t), x((pl.ds(0, 2), g), t) + y((pl.ds(0, 1), g), t)
        return fn

    wo_hbm, wo_buf = (wob_hbm, woa_hbm), (wob_buf, woa_buf)

    def wo_last(t, g):
        rows = lambda a, n: views(wo_hbm[g], wo_buf[g], (t >> 1, t & 1), [((pl.ds(a, n),),) * 2])
        return rows(992, 32), rows(896, 96)

    always = lambda g: True
    s_wa = Stream(32, cross(gather_piece(wuk_hbm, wuk_buf), gather_piece(wq_hbm, wq_buf)), always)
    s_wqb = Stream(16, lambda t, g: quad(wqb_piece, t, pre=(g,)))
    s_wuv = Stream(16, lambda t, g: quad(gather_piece(wuv_hbm, wuv_buf), t + 16 * g),
                   lambda g: g == 0)
    s_c = Stream(64, lambda t, g: quad(c_piece, t, post=(g,)))
    kv_stream = lambda hbm, buf, o: Stream(
        32, lambda t, g: quad(kv_piece(hbm.at[g, o & 1, :, o >> 1], buf.at[:, g]), t), always)
    k_stream = lambda o: kv_stream(k_hbm, k_buf, o)
    v_stream = lambda o: kv_stream(v_hbm, v_buf, o)
    s_wo = Stream(28, cross(wob_piece, woa_piece))
    s_wo_last = Stream(4, wo_last)

    def issue(cur, nxt, t, g, skip0=False):
        u = t + _LOOK
        _when(u < cur.steps, t > 0 if skip0 else True)(lambda: cur.start(u, g))
        for cond, st in nxt:
            _when(u >= cur.steps, cond)(lambda st=st: st.start(u - cur.steps, g, maybe0=True))

    def pace(cur, nxt, t, g):
        wait(t, g)
        issue(cur, nxt, t, g)

    def head_pair(buf, a, s, lo, hi):
        wp = _PITCH // 2
        lead = (slice(None),) * (len(buf.shape) - 2)
        reg = (lambda r: (r,)) if len(lead) == 1 else (lambda r: (r // 2, r % 2))
        words = buf.bitcast(jnp.uint32)
        n = 31 * wp + 52
        view = words.at[lead + (_ds(4 * a + 4, n, 4),)]
        last = words.at[lead + (_ds(4 * a + 4 + 4 * ((a + 1) >> 2), n, 4),)]
        x = jnp.concatenate(
            [(view if ml < 3 else last)[reg(r) + (pl.ds(16 * ml + s, 32, stride=wp), slice(None))]
             for r in range(lo, hi) for ml in range(4)], axis=0)
        even = pltpu.bitcast(x << 16, _F32).astype(_BF16)
        odd = pltpu.bitcast(x & jnp.uint32(0xFFFF0000), _F32).astype(_BF16)
        return even, odd

    units = [copies(s_wa.fn(t, g), t, g) for t in range(_LOOK) for g in range(2)]
    for c in units[0][0]:
        c.start(priority=0)
    for _, los in units:
        for c in los:
            c.start(priority=1)
    cxa = pltpu.make_async_copy(xa_hbm, xa_buf, xsem.at[0])
    cxb = pltpu.make_async_copy(xb_hbm, xb_buf, xsem.at[1])
    cxa.start()
    cxb.start()

    ji = lax.broadcasted_iota(jnp.int32, (1, 128), 1)
    src_row = 4 * (ji & 31) + (ji >> 5)

    def perm_row(m, c):
        perm_s[pl.ds(m, 1), :] = jnp.where(src_row == m, 1.0, 0.0)
        return c
    for k in range(8):
        lax.fori_loop(16 * k, 16 * k + 16, perm_row, 0)
        if k < 7:
            for c in units[k + 1][0]:
                c.start(priority=0)

    def clear(row):
        wq_buf[:, :, _ds(row, 8), :] = jnp.zeros((2, 2, 8, 128), _BF16)
        wuk_buf[:, :, _ds(row, 8), :] = jnp.zeros((2, 2, 8, 128), _BF16)
        wuv_buf[:, _ds(row, 8), :] = jnp.zeros((4, 8, 128), _BF16)

    def pa(t, c):
        for g in range(2):
            pace(s_wa, [(True, s_wqb)], t, g)
        clear(jnp.maximum(t * _PITCH - 8, 0))
        for ref in (qb_s, ob_s, rl_s, ctx_s):
            ref[_ds(t * 8, 8), :] = jnp.zeros((8, 128), _F32)
        for ref in (qabs_s, cc_s):
            ref[:, _ds(t * 8, 8), :] = jnp.zeros((4, 8, 128), _F32)
        return c
    lax.fori_loop(0, 32, pa, 0)
    clear(32 * _PITCH - 8)
    clear(32 * _PITCH + 8)
    cxa.wait()
    cxb.wait()
    perm = perm_s[...].astype(_BF16)
    xa = jnp.concatenate(
        [_dot(xa_buf[:, 128 * k:128 * (k + 1)], perm) for k in range(4)], axis=1).astype(_BF16)
    xb = xb_buf[...]
    ma_s[...] = jnp.full(ma_s.shape, -jnp.inf, _F32)

    def absorb(a, s, half):
        ev, od = head_pair(wuk_buf, a, s, 2 * half, 2 * half + 2)
        for h, w in ((8 * a + 2 * s, ev), (8 * a + 2 * s + 1, od)):
            r = _dot_nt(qa_s[h].astype(_BF16), w) * scale
            qabs_s[2 * half, _ds(h * 8, 4), :] = r[:, :128]
            qabs_s[2 * half + 1, _ds(h * 8, 4), :] = r[:, 128:]

    def p2(a, c):
        for s in range(4):
            t = 4 * a + s
            pace(s_wqb, [(True, s_wuv)], t, 0)
            ev, od = head_pair(wq_buf, a, s, 0, 4)
            qa_s[2 * t] = _dot(xa, ev)
            qa_s[2 * t + 1] = _dot(xa, od)
            pace(s_wqb, [(True, s_wuv)], t, 1)
            absorb(a, s, 0)
        return c
    lax.fori_loop(0, 4, p2, 0)

    def p3(a, c):
        for s in range(4):
            t = 4 * a + s
            pace(s_wuv, [(True, s_c)], t, 0)
            w = wqb_buf[:, :, :, _ds(t * 256, 256, 256)].reshape(512, 256)
            q = _dot(xb, w) * scale
            qb_s[_ds(t * 16, 4), :] = q[:, :128]
            qb_s[_ds(t * 16 + 8, 4), :] = q[:, 128:]
            pace(s_wuv, [(True, s_c)], t, 1)
            absorb(a, s, 1)
        return c
    lax.fori_loop(0, 4, p3, 0)

    nxt = [(True, k_stream(0))]

    def c_block(t, jb):
        return c_buf[t, pl.ds(2 * jb, 2)].reshape(128, 512)

    def c_scores(t, jb):
        b = 2 * (t >> 5) + jb
        sa = _dot_nt(qabs_t[_ds(b * 32, 32, 32), :], c_block(t, jb))
        sa_s[t, jb] = sa
        ma_s[b] = jnp.maximum(ma_s[b], sa)

    def unpermute(b0):
        for ct in range(4):
            r = jnp.concatenate(
                [qabs_s[ct, pl.ds(b, 32, stride=8), :] for b in (b0, b0 + 1)], axis=0)
            qabs_t[32 * b0:32 * b0 + 64, 128 * ct:128 * (ct + 1)] = (
                _dot_nt(r.astype(_BF16), perm).astype(_BF16))

    pace(s_c, nxt, 0, 0)
    unpermute(0)
    pace(s_c, nxt, 0, 1)
    unpermute(2)
    pace(s_c, nxt, 1, 0)
    q_rows = lambda o, i, g: pl.ds(32 * (2 * i + (o >> 1)) + (o & 1) + 2 * g, 4, stride=8)
    for o in range(4):
        for i in range(4):
            for g in range(2):
                qb_t[o, 8 * i + 4 * g:8 * i + 4 * g + 4, :] = qb_s[q_rows(o, i, g), :]

    def cstep(t, c):
        wait(t, 1)
        c_scores(t - 1, 0)
        issue(s_c, nxt, t, 1)
        wait(t + 1, 0)
        c_scores(t - 1, 1)
        issue(s_c, nxt, t + 1, 0)
        return c
    lax.fori_loop(1, 64, cstep, 0)
    c_scores(63, 0)
    c_scores(63, 1)

    top = lax.broadcasted_iota(jnp.int32, (8, 128), 0) < 4

    def batch(b, carry):
        ks, vs = k_stream(b), v_stream(b)
        qb = [qb_t[b, 8 * i:8 * i + 8, :].astype(_BF16) for i in range(4)]

        def kstep(t, mb):
            mb = list(mb)
            r = _ds(t * 128, 128, 128)
            se = [_dot_nt(qb[i], k_buf[i, 0, r, :]) for i in range(4)]
            issue(ks, [(True, vs)], t, 0, skip0=True)
            wait(t, 1)
            for i in range(4):
                s = jnp.where(top, se[i], _dot_nt(qb[i], k_buf[i, 1, r, :]))
                sb_s[t, i] = s
                mb[i] = jnp.maximum(mb[i], s)
            issue(ks, [(True, vs)], t, 1)
            wait(t + 1, 0)
            return tuple(mb)

        mb = lax.fori_loop(0, 32, kstep, (jnp.full((8, 128), -jnp.inf, _F32),) * 4)
        vs.start(_LOOK, 0)
        mb = [jnp.broadcast_to(jnp.max(m, axis=-1, keepdims=True), (8, 128)) for m in mb]
        ma = jnp.broadcast_to(jnp.max(ma_s[b], axis=-1, keepdims=True), (32, 128))

        nxt = [(b < 3, k_stream(jnp.minimum(b + 1, 3))), (b == 3, s_wo)]

        def vstep(t, c):
            lb, ab, la, aa = list(c[0]), list(c[1]), c[2], c[3]
            r = _ds(t * 128, 128, 128)
            issue(vs, nxt, t, 0, skip0=True)
            tc = (b >> 1) * 32 + t
            p = jnp.exp(sa_s[tc, b & 1] - ma)
            la = la + p
            aa = aa + _dot(p.astype(_BF16), c_block(tc, b & 1))
            wait(t, 1)
            for i in range(4):
                p = jnp.exp(sb_s[t, i] - mb[i])
                lb[i] = lb[i] + p
                p = p.astype(_BF16)
                ab[i] = ab[i] + jnp.where(top, _dot(p, v_buf[i, 0, r, :]),
                                          _dot(p, v_buf[i, 1, r, :]))
            issue(vs, nxt, t, 1)
            wait(t + 1, 0)
            return tuple(lb), tuple(ab), la, aa

        z8 = jnp.zeros((8, 128), _F32)
        lb, ab, la, aa = lax.fori_loop(
            0, 32, vstep,
            ((z8,) * 4, (z8,) * 4, jnp.zeros((32, 128), _F32), jnp.zeros((32, 512), _F32)))
        for cond, st in nxt:
            pl.when(cond)(lambda st=st: st.start(_LOOK, 0))
        ob = [ab[i] / jnp.sum(lb[i], axis=-1, keepdims=True) for i in range(4)]
        rl = jnp.broadcast_to(1.0 / jnp.sum(la, axis=-1, keepdims=True), (32, 128))
        aa = aa.astype(_BF16)
        cc = [_dot(aa[:, 128 * ct:128 * (ct + 1)], perm) for ct in range(4)]
        for bb in range(4):
            @pl.when(b == bb)
            def _():
                rows = pl.ds(bb, 32, stride=8)
                for i in range(4):
                    for g in range(2):
                        ob_s[q_rows(bb, i, g), :] = ob[i][4 * g:4 * g + 4]
                rl_s[rows, :] = rl
                for ct in range(4):
                    cc_s[ct, rows, :] = cc[ct]
        return carry
    lax.fori_loop(0, 4, batch, 0)

    lhs_of = (ob_s, ctx_s)

    def proj(g, rg, j):
        lhs = lhs_of[g][_ds((8 * rg + j) * 8, 4), :].astype(_BF16)
        return _dot(lhs, wo_buf[g][rg >> 1, rg & 1, _ds(j * 128, 128, 128), :])

    nxt = [(True, s_wo_last)]

    def fstep(s, gs):
        def body(t, out):
            rg, j = t & 3, (t >> 2) - 1
            out = tuple(out[g] + proj(g, rg, j) if g in gs else out[g] for g in range(2))
            issue(s_wo, nxt, t, 0, skip0=True)
            pace(s_wo, nxt, t, 1)
            if s is not None:
                ev, od = head_pair(wuv_buf, rg, s, 0, 4)
                for h, w in ((8 * rg + 2 * s, ev), (8 * rg + 2 * s + 1, od)):
                    row = _ds(h * 8, 4)
                    lhs = jnp.concatenate([cc_s[ct, row, :] for ct in range(4)], axis=1)
                    ctx_s[row, :] = _dot(lhs.astype(_BF16), w) * rl_s[row, :]
            wait(t + 1, 0)
            return out
        return body

    out = (jnp.zeros((4, 512), _F32),) * 2
    for k, s in enumerate((0, None, 1, None, 2, 3, None)):
        out = lax.fori_loop(4 * k, 4 * k + 4, fstep(s, {0: (), 1: (1,)}.get(k, (0, 1))), out)
    out = list(out)
    for rg in range(4):
        out[0] = out[0] + proj(0, rg, 6) + proj(0, rg, 0)
        out[1] = out[1] + proj(1, rg, 6)
    for u in range(8):
        for v in {1: (1, 2, 3, 4), 5: (5, 6), 7: (7,)}.get(u, ()):
            wait(v >> 1, v & 1)
        out[u & 1] = out[u & 1] + proj(u & 1, u >> 1, 7)
        if u == 6:
            out_ref[:, 512:] = out[0].astype(out_ref.dtype)
    out_ref[:, :512] = out[1].astype(out_ref.dtype)


@jax.jit
def pallas_concat_heads__compressed_kv_cla__gqa_block_cached__decode_kernel(
    A_x: jax.Array,
    A_c_kv: jax.Array,
    A_w_q: jax.Array,
    A_w_uk: jax.Array,
    A_w_uv: jax.Array,
    A_w_o: jax.Array,
    B_x: jax.Array,
    B_k_cache: jax.Array,
    B_v_cache: jax.Array,
    B_wq: jax.Array,
    B_wo: jax.Array,
):
    vm = pltpu.VMEM
    pitched = 32 * _PITCH + 16
    out = pl.pallas_call(
        _kernel,
        in_specs=[pl.BlockSpec(memory_space=pl.ANY)] * 11,
        out_specs=pl.BlockSpec(memory_space=pltpu.VMEM),
        out_shape=jax.ShapeDtypeStruct((4, 1024), _BF16),
        scratch_shapes=[
            vm((4, 512), _BF16),
            vm((4, 512), _BF16),
            vm((2, 2, pitched, 128), _BF16),
            vm((2, 2, pitched, 128), _BF16),
            vm((4, pitched, 128), _BF16),
            vm((2, 2, 1024, 512), _BF16),
            vm((2, 4, 64, 4096), _BF16),
            vm((2, 2, 1024, 512), _BF16),
            vm((64, 4, 2, 32, 512), _BF16),
            vm((4, 2, 4096, 128), _BF16),
            vm((4, 2, 4096, 128), _BF16),
            vm((3, 128, 128), _BF16),
            vm((128, 128), _F32),
            vm((32, 4, 128), _F32),
            vm((4, 256, 128), _F32),
            vm((128, 512), _BF16),
            vm((256, 128), _F32),
            vm((4, 32, 128), _F32),
            vm((64, 2, 32, 128), _F32),
            vm((4, 32, 128), _F32),
            vm((32, 4, 8, 128), _F32),
            vm((256, 128), _F32),
            vm((4, 256, 128), _F32),
            vm((256, 128), _F32),
            vm((256, 128), _F32),
            pltpu.SemaphoreType.DMA((_LOOK * 2,)),
            pltpu.SemaphoreType.DMA((_LOOK * 2,)),
            pltpu.SemaphoreType.DMA((2,)),
        ],
        compiler_params=pltpu.CompilerParams(
            vmem_limit_bytes=80 * 1024 * 1024,
            disable_bounds_checks=True,
            disable_semaphore_checks=True),
    )(
        A_x.reshape(4, 512), A_c_kv.reshape(2, 4, 2, 1024, 512),
        A_w_q.reshape(2, 2, 4096, 128), A_w_uk.reshape(2, 2, 4096, 128),
        A_w_uv.reshape(4, 4096, 128), A_w_o.reshape(2, 2, 1024, 512),
        B_x.reshape(4, 512), B_k_cache.reshape(2, 2, 4, 2, 4096, 128),
        B_v_cache.reshape(2, 2, 4, 2, 4096, 128),
        B_wq.reshape(2, 4, 64, 4096), B_wo.reshape(2, 2, 1024, 512),
    )
    return out.reshape(4, 1, 1024)
```
